```python
import jax
import jax.numpy as jnp

def _softmax(x, axis=-1):
    return jax.nn.softmax(x, axis=axis)

def _gelu(x):
    return jax.nn.gelu(x, approximate=True)

def _silu(x):
    return jax.nn.silu(x)

def _sigmoid(x):
    return jax.nn.sigmoid(x)

def _layernorm(x, axis=-1, eps=1e-05):
    m = jnp.mean(x, axis=axis, keepdims=True)
    v = jnp.var(x, axis=axis, keepdims=True)
    return (x - m) / jnp.sqrt(v + eps)

def _scatter_add(tgt, idx, src, axis=0):
    return tgt.at[idx].add(src)

def _segment_sum(src, seg, n):
    return jax.ops.segment_sum(src, seg, n)

class _Rng:

    def __init__(self, key):
        self._k = key

    def _next(self):
        self._k, sub = jax.random.split(self._k)
        return sub

    def normal(self, shape):
        return jax.random.normal(self._next(), shape, dtype=jnp.bfloat16)

    def randint(self, lo, hi, shape):
        return jax.random.randint(self._next(), shape, lo, hi, dtype=jnp.int32)

    def uniform(self, shape, lo=0.0, hi=1.0):
        return jax.random.uniform(self._next(), shape, jnp.bfloat16, lo, hi)

    def permutation(self, n):
        return jax.random.permutation(self._next(), n)
kernel_name = 'interleave_layers__memory_aug_infini_attn__mixer_s_mlp__prompt'

def setup_inputs():
    _rng = _Rng(jax.random.key(int.from_bytes(__import__("os").urandom(4), "little")))
    _w = lambda a: (lambda t: t.astype(jnp.bfloat16) if jnp.issubdtype(t.dtype, jnp.floating) else t)(jnp.asarray(a))

    def _A_setup():
        B, S, D, H = (1, 2048, 1024, 32)
        N = 4
        L = max(1, S // N)
        sc = D ** (-0.5)
        return {'x': _w((lambda *s: _rng.normal(s) * 0.05)(B, N * L, D)), 'wq': _w((lambda *s: _rng.normal(s) * 0.05)(D, D) * sc), 'wk': _w((lambda *s: _rng.normal(s) * 0.05)(D, D) * sc), 'wv': _w((lambda *s: _rng.normal(s) * 0.05)(D, D) * sc), 'wo': _w((lambda *s: _rng.normal(s) * 0.05)(D, D) * sc), 'beta': _w((lambda *s: _rng.normal(s) * 0.05)(H))}
    _A_in = _A_setup()

    def _B_setup():
        B, S, D, F = (1, 2048, 1024, 3584)
        return {'x': _w((lambda *s: _rng.normal(s) * 0.05)(B, S, D)), 'w1': _w((lambda *s: _rng.normal(s) * 0.05)(D, D) * D ** (-0.5)), 'w2': _w((lambda *s: _rng.normal(s) * 0.05)(D, D) * D ** (-0.5)), 'w3': _w((lambda *s: _rng.normal(s) * 0.05)(D, F) * D ** (-0.5)), 'w4': _w((lambda *s: _rng.normal(s) * 0.05)(F, D) * F ** (-0.5))}
    _B_in = _B_setup()
    return {'A_x': _A_in['x'], 'A_wq': _A_in['wq'], 'A_wk': _A_in['wk'], 'A_wv': _A_in['wv'], 'A_wo': _A_in['wo'], 'A_beta': _A_in['beta'], 'B_x': _B_in['x'], 'B_w1': _B_in['w1'], 'B_w2': _B_in['w2'], 'B_w3': _B_in['w3'], 'B_w4': _B_in['w4']}

def reference(A_x, A_wq, A_wk, A_wv, A_wo, A_beta, B_x, B_w1, B_w2, B_w3, B_w4):

    def _A_ref(x, wq, wk, wv, wo, beta):
        B, S, D = x.shape
        H = 32
        Dh = D // H
        N = 4
        L = S // N
        q = (lambda x, *d: x.transpose(*d))((x @ wq).reshape(B, S, H, Dh), 0, 2, 1, 3).reshape(B, H, N, L, Dh)
        k = (lambda x, *d: x.transpose(*d))((x @ wk).reshape(B, S, H, Dh), 0, 2, 1, 3).reshape(B, H, N, L, Dh)
        v = (lambda x, *d: x.transpose(*d))((x @ wv).reshape(B, S, H, Dh), 0, 2, 1, 3).reshape(B, H, N, L, Dh)
        phi = lambda t: jnp.where(t > 0, t + 1.0, jnp.exp(t))
        scale = Dh ** (-0.5)
        ar = jnp.arange(L)
        mask = (lambda x, dt: x.astype(dt))(ar[:, None] < ar[None, :], x.dtype) * -1000000000.0
        g = _sigmoid(beta).reshape(1, H, 1, 1)
        M = jnp.einsum('bhd,bhe->bhde', q[:, :, 0, 0, :] * 0.0, q[:, :, 0, 0, :] * 0.0)
        z = q[:, :, 0, 0, :] * 0.0
        outs = []
        for s in range(N):
            qs, ks, vs = (q[:, :, s].copy(), k[:, :, s].copy(), v[:, :, s].copy())
            logits = jnp.einsum('bhqd,bhkd->bhqk', qs, ks) * scale + mask
            p = _softmax(logits, axis=-1)
            a_dot = jnp.einsum('bhqk,bhkd->bhqd', p, vs)
            pq = phi(qs)
            num = jnp.einsum('bhld,bhde->bhle', pq, M)
            den = jnp.einsum('bhld,bhd->bhl', pq, z)[..., None] + 1e-06
            a_mem = num / den
            o = g * a_mem + (1.0 - g) * a_dot
            outs.append(o)
            pk = phi(ks)
            M = M + jnp.einsum('bhld,bhle->bhde', pk, vs)
            z = z + jnp.einsum('bhld->bhd', pk)
        o = (lambda x, *d: x.transpose(*d))(jnp.stack(outs, 2).reshape(B, H, S, Dh), 0, 2, 1, 3).reshape(B, S, D)
        return o @ wo

    def _B_ref(x, w1, w2, w3, w4):
        B, S, D = x.shape
        h = _gelu(_layernorm(x, axis=-1) @ w1)
        c = D // 4
        g0 = jnp.pad(h[:, :, 0 * c:1 * c], ((0, 0), (1, 0), (0, 0)))[:, :S, :]
        g1 = jnp.pad(h[:, :, 1 * c:2 * c], ((0, 0), (0, 1), (0, 0)))[:, 1:, :]
        g2 = jnp.pad(h[:, :, 2 * c:3 * c], ((0, 0), (2, 0), (0, 0)))[:, :S, :]
        g3 = jnp.pad(h[:, :, 3 * c:], ((0, 0), (0, 2), (0, 0)))[:, 2:, :]
        hs = jnp.concatenate([g0, g1, g2, g3], axis=-1) @ w2
        x1 = x + hs
        h2 = _gelu(_layernorm(x1, axis=-1) @ w3) @ w4
        return x1 + h2
    x = A_x
    x = x + _A_ref(_layernorm(x, axis=-1), A_wq, A_wk, A_wv, A_wo, A_beta)
    x = x + _B_ref(_layernorm(x, axis=-1), B_w1, B_w2, B_w3, B_w4)
    x = x + _A_ref(_layernorm(x, axis=-1), A_wq, A_wk, A_wv, A_wo, A_beta)
    x = x + _B_ref(_layernorm(x, axis=-1), B_w1, B_w2, B_w3, B_w4)
    return x
```

```python
import functools

import jax
import jax.numpy as jnp
from jax import lax
import jax.experimental.pallas as pl
import jax.experimental.pallas.tpu as pltpu

S = 2048
D = 1024
H = 32
DH = 32
NSEG = 4
L = 512
F = 3584
G = 8
HPG = 4
QT = 128
NQT = L // QT
HPAD = 8
FC = 512

LOG2E = 1.4426950408889634
QSCALE = (DH ** -0.5) * LOG2E
MASK_BIAS = -1000000000.0 * LOG2E
GELU_C = 0.7978845608028654

F32 = jnp.float32
BF16 = jnp.bfloat16

NT = (((1,), (1,)), ((), ()))


def _ln(x):
    m = jnp.mean(x, axis=-1, keepdims=True)
    d = x - m
    v = jnp.mean(d * d, axis=-1, keepdims=True)
    return d * lax.rsqrt(v + 1e-05)


def _gelu(x):
    return 0.5 * x * (1.0 + jnp.tanh(GELU_C * (x + 0.044715 * (x * x * x))))


def _phi(t):
    return jnp.where(t > 0, t + 1.0, jnp.exp(t))


def _dot(a, b):
    return jnp.dot(a, b, preferred_element_type=F32)


def _kernel(beta_ref, x_hbm, wq_hbm, wk_hbm, wv_hbm, wo_hbm, w1_hbm, w2_hbm, w3_hbm, w4_hbm,
            out_hbm,
            xin, wq, wk, wv, wo, w1, w2, w3, w4, wqvt,
            xres, ybuf, hbuf, kb, pkb, qt, pqt, vt, ob, mt, zr, obuf,
            sem_in, sem_out):

    def x_copy(s):
        return pltpu.make_async_copy(x_hbm.at[pl.ds(s * L, L)], xin.at[pl.ds(s * L, L)], sem_in.at[s])

    w_pairs = [(wk_hbm, wk), (wq_hbm, wq), (wv_hbm, wv), (wo_hbm, wo), (w1_hbm, w1),
               (w2_hbm, w2), (w3_hbm, w3), (w4_hbm, w4)]
    w_copies = [pltpu.make_async_copy(src, dst, sem_in.at[NSEG + i])
                for i, (src, dst) in enumerate(w_pairs)]
    cp_wk, cp_wq, cp_wv, cp_wo, cp_w1, cp_w2, cp_w3, cp_w4 = w_copies

    x_copy(0).start()
    cp_wk.start()
    cp_wq.start()
    cp_wv.start()
    for s in range(1, NSEG):
        x_copy(s).start()
    for cp in (cp_wo, cp_w1, cp_w2, cp_w3, cp_w4):
        cp.start()

    hbuf[0:HPAD, :] = jnp.zeros((HPAD, D), F32)
    hbuf[HPAD + S:HPAD + S + HPAD, :] = jnp.zeros((HPAD, D), F32)

    def attn_group(g):
        r0 = pl.multiple_of(g * 128, 128)
        kg = kb[g]
        qg = qt[pl.ds(r0, 128), :]
        vg = vt[pl.ds(r0, 128), :]

        krow = lax.broadcasted_iota(jnp.int32, (QT, QT), 0)
        qcol = lax.broadcasted_iota(jnp.int32, (QT, QT), 1)
        bias = jnp.where(krow > qcol, MASK_BIAS, 0.0).astype(F32)
        bias4 = jnp.concatenate([bias] * HPG, axis=1)

        mem = jnp.concatenate([mt[g], zr[g]], axis=0).astype(BF16)
        nd = _dot(mem, pqt[pl.ds(r0, 128), :])

        zero_blk = jnp.zeros((DH, QT), BF16)
        od = [[None] * NQT for _ in range(HPG)]
        ls = [None] * NQT
        for i in reversed(range(NQT)):
            nk = QT * (i + 1)
            qi = qg[:, i * QT:(i + 1) * QT]
            cols = []
            for h in range(HPG):
                blocks = [zero_blk] * HPG
                blocks[h] = qi[h * DH:(h + 1) * DH, :]
                cols.append(jnp.concatenate(blocks, axis=0))
            qbd = jnp.concatenate(cols, axis=1)
            st = _dot(kg[:nk, :], qbd)
            diag = st[nk - QT:, :] + bias4
            st = diag if i == 0 else jnp.concatenate([st[:nk - QT, :], diag], axis=0)
            m = jnp.max(st, axis=0, keepdims=True)
            p = jnp.exp2(st - m)
            ls[i] = jnp.sum(p, axis=0, keepdims=True)
            pb = p.astype(BF16)
            for h in range(HPG):
                od[h][i] = _dot(vg[h * DH:(h + 1) * DH, :nk], pb[:, h * QT:(h + 1) * QT])

        rows = []
        for h in range(HPG):
            gate = jax.nn.sigmoid(jnp.full((1, L), beta_ref[g * HPG + h], F32))
            l_h = jnp.concatenate([ls[i][:, h * QT:(h + 1) * QT] for i in range(NQT)], axis=1)
            c_dot = (1.0 - gate) / l_h
            c_mem = gate / (nd[128 + h:129 + h, :] + 1e-06)
            o_h = jnp.concatenate(od[h], axis=1)
            rows.append(c_mem * nd[h * DH:(h + 1) * DH, :] + c_dot * o_h)
        ot = jnp.concatenate(rows, axis=0)
        ob[g] = ot.T.astype(BF16)

        vaug = jnp.concatenate([vg, jnp.ones((16, L), BF16)], axis=0)
        upd = _dot(vaug, pkb[g])
        rh = lax.broadcasted_iota(jnp.int32, (128, 128), 0) // DH
        ch = lax.broadcasted_iota(jnp.int32, (128, 128), 1) // DH
        mt[g] = mt[g] + jnp.where(rh == ch, upd[:128, :], 0.0)
        zrh = lax.broadcasted_iota(jnp.int32, (16, 128), 0)
        zch = lax.broadcasted_iota(jnp.int32, (16, 128), 1) // DH
        zr[g] = zr[g] + jnp.where(zrh == zch, upd[128:, :], 0.0)

    def a_step(s, first):
        r = s * L if first else pl.multiple_of(s * L, L)
        if first:
            x_copy(0).wait()
            x = xin[0:L, :].astype(F32)
            cp_wk.wait()
        else:
            x = xres[pl.ds(r, L), :]
        xn = _ln(x).astype(BF16)
        k = _dot(xn, wk[...])
        pk = _phi(k).astype(BF16)
        k = k.astype(BF16)
        for g in range(G):
            kb[g] = k[:, g * 128:(g + 1) * 128]
            pkb[g] = pk[:, g * 128:(g + 1) * 128]
        if first:
            cp_wq.wait()
            cp_wv.wait()
            wqvt[0:D, :] = wq[...].T
            wqvt[D:2 * D, :] = wv[...].T
        qv = lax.dot_general(wqvt[...], xn, NT, preferred_element_type=F32)
        q = qv[:D, :]
        qt[...] = (q * QSCALE).astype(BF16)
        pqt[...] = _phi(q).astype(BF16)
        vt[...] = qv[D:, :].astype(BF16)
        if first:
            for s2 in range(1, NSEG):
                x_copy(s2).wait()
                xres[s2 * L:(s2 + 1) * L, :] = xin[s2 * L:(s2 + 1) * L, :].astype(F32)

        def group_body(g, c):
            attn_group(g)
            return c
        lax.fori_loop(0, G, group_body, 0)

        if first:
            cp_wo.wait()
            cp_w1.wait()
            x = xin[0:L, :].astype(F32)
        else:
            x = xres[pl.ds(r, L), :]
        o = jnp.concatenate([ob[g] for g in range(G)], axis=1)
        xm = x + _dot(o, wo[...])
        xres[pl.ds(r, L), :] = xm
        y = _ln(xm)
        ybuf[pl.ds(r, L), :] = y
        yn = _ln(y).astype(BF16)
        hr = HPAD + r if first else pl.multiple_of(HPAD + r, HPAD)
        hbuf[pl.ds(hr, L), :] = _gelu(_dot(yn, w1[...]))

    def out_copy(t, slot):
        return pltpu.make_async_copy(obuf.at[slot], out_hbm.at[pl.ds(t * L, L)], sem_out.at[slot])

    def b_step(t, layer):
        r = pl.multiple_of(t * L, L)
        c = D // 4
        win = hbuf[pl.ds(r, L + 2 * HPAD), :]
        parts = []
        for ci, off in enumerate((-1, 1, -2, 2)):
            parts.append(win[HPAD + off:HPAD + off + L, ci * c:(ci + 1) * c].astype(BF16))
        gsh = jnp.concatenate(parts, axis=1)
        x1 = ybuf[pl.ds(r, L), :] + _dot(gsh, w2[...])
        xn = _ln(x1).astype(BF16)
        acc = xres[pl.ds(r, L), :] + x1
        for ci in range(F // FC):
            h = _gelu(_dot(xn, w3[:, ci * FC:(ci + 1) * FC])).astype(BF16)
            acc = acc + _dot(h, w4[ci * FC:(ci + 1) * FC, :])
        xres[pl.ds(r, L), :] = acc

        @pl.when(layer == 1)
        def _():
            obuf[t] = xres[pl.ds(r, L), :].astype(BF16)
            out_copy(t, t).start()

    def reset_memory():
        mt[...] = jnp.zeros(mt.shape, F32)
        zr[...] = jnp.zeros(zr.shape, F32)

    reset_memory()
    a_step(0, True)

    def step(i, c):
        layer = i // (2 * NSEG)
        j = i % (2 * NSEG)

        @pl.when(j == 0)
        def _():
            reset_memory()

        @pl.when(i == NSEG)
        def _():
            cp_w2.wait()
            cp_w3.wait()
            cp_w4.wait()

        @pl.when(j < NSEG)
        def _():
            a_step(j, False)

        @pl.when(j >= NSEG)
        def _():
            b_step(j - NSEG, layer)
        return c

    lax.fori_loop(1, 4 * NSEG, step, 0)

    for t in range(NSEG):
        out_copy(t, t).wait()


@jax.jit
def pallas_interleave_layers__memory_aug_infini_attn__mixer_s_mlp__prompt_kernel(
    A_x: jax.Array,
    A_wq: jax.Array,
    A_wk: jax.Array,
    A_wv: jax.Array,
    A_wo: jax.Array,
    A_beta: jax.Array,
    B_x: jax.Array,
    B_w1: jax.Array,
    B_w2: jax.Array,
    B_w3: jax.Array,
    B_w4: jax.Array,
):
    del B_x
    x = A_x.reshape(S, D)
    beta = A_beta.astype(F32)
    any_spec = pl.BlockSpec(memory_space=pl.ANY)
    scratch = [
        pltpu.VMEM((S, D), BF16),
        pltpu.VMEM((D, D), BF16),
        pltpu.VMEM((D, D), BF16),
        pltpu.VMEM((D, D), BF16),
        pltpu.VMEM((D, D), BF16),
        pltpu.VMEM((D, D), BF16),
        pltpu.VMEM((D, D), BF16),
        pltpu.VMEM((D, F), BF16),
        pltpu.VMEM((F, D), BF16),
        pltpu.VMEM((2 * D, D), BF16),
        pltpu.VMEM((S, D), F32),
        pltpu.VMEM((S, D), F32),
        pltpu.VMEM((S + 2 * HPAD, D), F32),
        pltpu.VMEM((G, L, 128), BF16),
        pltpu.VMEM((G, L, 128), BF16),
        pltpu.VMEM((D, L), BF16),
        pltpu.VMEM((D, L), BF16),
        pltpu.VMEM((D, L), BF16),
        pltpu.VMEM((G, L, 128), BF16),
        pltpu.VMEM((G, 128, 128), F32),
        pltpu.VMEM((G, 16, 128), F32),
        pltpu.VMEM((NSEG, L, D), BF16),
        pltpu.SemaphoreType.DMA((NSEG + 8,)),
        pltpu.SemaphoreType.DMA((NSEG,)),
    ]
    out = pl.pallas_call(
        _kernel,
        out_shape=jax.ShapeDtypeStruct((S, D), BF16),
        in_specs=[pl.BlockSpec(memory_space=pltpu.SMEM)] + [any_spec] * 9,
        out_specs=any_spec,
        scratch_shapes=scratch,
        compiler_params=pltpu.CompilerParams(vmem_limit_bytes=120 * 1024 * 1024),
    )(beta, x, A_wq, A_wk, A_wv, A_wo, B_w1, B_w2, B_w3, B_w4)
    return out.reshape(1, S, D)
```

```python
import functools

import jax
import jax.numpy as jnp
from jax import lax
import jax.experimental.pallas as pl
import jax.experimental.pallas.tpu as pltpu

S = 2048
D = 1024
H = 32
DH = 32
NSEG = 4
L = 512
F = 3584
G = 8
HPG = 4
QT = 128
NQT = L // QT
HPAD = 8
FC = 512

LOG2E = 1.4426950408889634
QSCALE = (DH ** -0.5) * LOG2E
MASK_BIAS = -1000000000.0 * LOG2E
GELU_C = 0.7978845608028654

F32 = jnp.float32
BF16 = jnp.bfloat16

NT = (((1,), (1,)), ((), ()))


def _ln(x):
    m = jnp.mean(x, axis=-1, keepdims=True)
    d = x - m
    v = jnp.mean(d * d, axis=-1, keepdims=True)
    return d * lax.rsqrt(v + 1e-05)


def _gelu(x):
    return 0.5 * x * (1.0 + jnp.tanh(GELU_C * (x + 0.044715 * (x * x * x))))


def _phi(t):
    return jnp.where(t > 0, t + 1.0, jnp.exp(t))


def _dot(a, b):
    return jnp.dot(a, b, preferred_element_type=F32)


def _kernel(beta_ref, x_hbm, wq_hbm, wk_hbm, wv_hbm, wo_hbm, w1_hbm, w2_hbm, w3_hbm, w4_hbm,
            out_hbm,
            xin, wq, wk, wv, wo, w1, w2, w3, w4, wqvt,
            xres, ybuf, hbuf, kb, pkb, qt, pqt, vt, ob, mt, zr, obuf,
            sem_in, sem_out):

    def x_copy(s):
        return pltpu.make_async_copy(x_hbm.at[pl.ds(s * L, L)], xin.at[pl.ds(s * L, L)], sem_in.at[s])

    w_pairs = [(wk_hbm, wk), (wq_hbm, wq), (wv_hbm, wv), (wo_hbm, wo), (w1_hbm, w1),
               (w2_hbm, w2), (w3_hbm, w3), (w4_hbm, w4)]
    w_copies = [pltpu.make_async_copy(src, dst, sem_in.at[NSEG + i])
                for i, (src, dst) in enumerate(w_pairs)]
    cp_wk, cp_wq, cp_wv, cp_wo, cp_w1, cp_w2, cp_w3, cp_w4 = w_copies

    x_copy(0).start()
    cp_wk.start()
    cp_wq.start()
    cp_wv.start()
    for s in range(1, NSEG):
        x_copy(s).start()
    for cp in (cp_wo, cp_w1, cp_w2, cp_w3, cp_w4):
        cp.start()

    hbuf[0:HPAD, :] = jnp.zeros((HPAD, D), F32)
    hbuf[HPAD + S:HPAD + S + HPAD, :] = jnp.zeros((HPAD, D), F32)

    def attn_group(g):
        r0 = pl.multiple_of(g * 128, 128)
        kg = kb[g]
        qg = qt[pl.ds(r0, 128), :]
        vg = vt[pl.ds(r0, 128), :]

        krow = lax.broadcasted_iota(jnp.int32, (QT, QT), 0)
        qcol = lax.broadcasted_iota(jnp.int32, (QT, QT), 1)
        bias = jnp.where(krow > qcol, MASK_BIAS, 0.0).astype(F32)
        bias4 = jnp.concatenate([bias] * HPG, axis=1)

        mem = jnp.concatenate([mt[g], zr[g]], axis=0).astype(BF16)
        nd = _dot(mem, pqt[pl.ds(r0, 128), :])

        zero_blk = jnp.zeros((DH, QT), BF16)
        od = [[None] * NQT for _ in range(HPG)]
        ls = [None] * NQT
        for i in reversed(range(NQT)):
            nk = QT * (i + 1)
            qi = qg[:, i * QT:(i + 1) * QT]
            cols = []
            for h in range(HPG):
                blocks = [zero_blk] * HPG
                blocks[h] = qi[h * DH:(h + 1) * DH, :]
                cols.append(jnp.concatenate(blocks, axis=0))
            qbd = jnp.concatenate(cols, axis=1)
            st = _dot(kg[:nk, :], qbd)
            diag = st[nk - QT:, :] + bias4
            st = diag if i == 0 else jnp.concatenate([st[:nk - QT, :], diag], axis=0)
            m = jnp.max(st, axis=0, keepdims=True)
            p = jnp.exp2(st - m)
            ls[i] = jnp.sum(p, axis=0, keepdims=True)
            pb = p.astype(BF16)
            for h in range(HPG):
                od[h][i] = _dot(vg[h * DH:(h + 1) * DH, :nk], pb[:, h * QT:(h + 1) * QT])

        rows = []
        for h in range(HPG):
            gate = jax.nn.sigmoid(jnp.full((1, L), beta_ref[g * HPG + h], F32))
            l_h = jnp.concatenate([ls[i][:, h * QT:(h + 1) * QT] for i in range(NQT)], axis=1)
            c_dot = (1.0 - gate) / l_h
            c_mem = gate / (nd[128 + h:129 + h, :] + 1e-06)
            o_h = jnp.concatenate(od[h], axis=1)
            rows.append(c_mem * nd[h * DH:(h + 1) * DH, :] + c_dot * o_h)
        ot = jnp.concatenate(rows, axis=0)
        ob[g] = ot.T.astype(BF16)

        vaug = jnp.concatenate([vg, jnp.ones((16, L), BF16)], axis=0)
        upd = _dot(vaug, pkb[g])
        rh = lax.broadcasted_iota(jnp.int32, (128, 128), 0) // DH
        ch = lax.broadcasted_iota(jnp.int32, (128, 128), 1) // DH
        mt[g] = mt[g] + jnp.where(rh == ch, upd[:128, :], 0.0)
        zrh = lax.broadcasted_iota(jnp.int32, (16, 128), 0)
        zch = lax.broadcasted_iota(jnp.int32, (16, 128), 1) // DH
        zr[g] = zr[g] + jnp.where(zrh == zch, upd[128:, :], 0.0)

    def a_step(s, first):
        r = s * L if first else pl.multiple_of(s * L, L)
        if first:
            x_copy(0).wait()
            x = xin[0:L, :].astype(F32)
            cp_wk.wait()
        else:
            x = xres[pl.ds(r, L), :]
        xn = _ln(x).astype(BF16)
        k = _dot(xn, wk[...])
        pk = _phi(k).astype(BF16)
        k = k.astype(BF16)
        for g in range(G):
            kb[g] = k[:, g * 128:(g + 1) * 128]
            pkb[g] = pk[:, g * 128:(g + 1) * 128]
        if first:
            cp_wq.wait()
            cp_wv.wait()
            wqvt[0:D, :] = wq[...].T
            wqvt[D:2 * D, :] = wv[...].T
        qv = lax.dot_general(wqvt[...], xn, NT, preferred_element_type=F32)
        q = qv[:D, :]
        qt[...] = (q * QSCALE).astype(BF16)
        pqt[...] = _phi(q).astype(BF16)
        vt[...] = qv[D:, :].astype(BF16)
        if first:
            for s2 in range(1, NSEG):
                x_copy(s2).wait()
                xres[s2 * L:(s2 + 1) * L, :] = xin[s2 * L:(s2 + 1) * L, :].astype(F32)

        def group_body(g, c):
            attn_group(g)
            return c
        lax.fori_loop(0, G, group_body, 0)

        if first:
            cp_wo.wait()
            cp_w1.wait()
            x = xin[0:L, :].astype(F32)
        else:
            x = xres[pl.ds(r, L), :]
        o = jnp.concatenate([ob[g] for g in range(G)], axis=1)
        xm = x + _dot(o, wo[...])
        xres[pl.ds(r, L), :] = xm
        y = _ln(xm)
        ybuf[pl.ds(r, L), :] = y
        yn = _ln(y).astype(BF16)
        hr = HPAD + r if first else pl.multiple_of(HPAD + r, HPAD)
        hbuf[pl.ds(hr, L), :] = _gelu(_dot(yn, w1[...]))

    def out_copy(t, slot):
        return pltpu.make_async_copy(obuf.at[slot], out_hbm.at[pl.ds(t * L, L)], sem_out.at[slot])

    def b_step(t, layer):
        r = pl.multiple_of(t * L, L)
        c = D // 4
        win = hbuf[pl.ds(r, L + 2 * HPAD), :]
        parts = []
        for ci, off in enumerate((-1, 1, -2, 2)):
            parts.append(win[HPAD + off:HPAD + off + L, ci * c:(ci + 1) * c].astype(BF16))
        gsh = jnp.concatenate(parts, axis=1)
        x1 = ybuf[pl.ds(r, L), :] + _dot(gsh, w2[...])
        xn = _ln(x1).astype(BF16)
        acc = xres[pl.ds(r, L), :] + x1
        for ci in range(F // FC):
            h = _gelu(_dot(xn, w3[:, ci * FC:(ci + 1) * FC])).astype(BF16)
            acc = acc + _dot(h, w4[ci * FC:(ci + 1) * FC, :])
        xres[pl.ds(r, L), :] = acc

        @pl.when(layer == 1)
        def _():
            obuf[t] = xres[pl.ds(r, L), :].astype(BF16)
            out_copy(t, t).start()

    def reset_memory():
        mt[...] = jnp.zeros(mt.shape, F32)
        zr[...] = jnp.zeros(zr.shape, F32)

    reset_memory()
    a_step(0, True)

    def layer_body(layer, c):
        def a_body(j, c2):
            a_step(j, False)
            return c2
        lax.fori_loop(1 - layer, NSEG, a_body, 0)

        @pl.when(layer == 0)
        def _():
            cp_w2.wait()
            cp_w3.wait()
            cp_w4.wait()

        def b_body(t, c2):
            b_step(t, layer)
            return c2
        lax.fori_loop(0, NSEG, b_body, 0)
        reset_memory()
        return c

    lax.fori_loop(0, 2, layer_body, 0)

    for t in range(NSEG):
        out_copy(t, t).wait()


@jax.jit
def pallas_interleave_layers__memory_aug_infini_attn__mixer_s_mlp__prompt_kernel(
    A_x: jax.Array,
    A_wq: jax.Array,
    A_wk: jax.Array,
    A_wv: jax.Array,
    A_wo: jax.Array,
    A_beta: jax.Array,
    B_x: jax.Array,
    B_w1: jax.Array,
    B_w2: jax.Array,
    B_w3: jax.Array,
    B_w4: jax.Array,
):
    del B_x
    x = A_x.reshape(S, D)
    beta = A_beta.astype(F32)
    any_spec = pl.BlockSpec(memory_space=pl.ANY)
    scratch = [
        pltpu.VMEM((S, D), BF16),
        pltpu.VMEM((D, D), BF16),
        pltpu.VMEM((D, D), BF16),
        pltpu.VMEM((D, D), BF16),
        pltpu.VMEM((D, D), BF16),
        pltpu.VMEM((D, D), BF16),
        pltpu.VMEM((D, D), BF16),
        pltpu.VMEM((D, F), BF16),
        pltpu.VMEM((F, D), BF16),
        pltpu.VMEM((2 * D, D), BF16),
        pltpu.VMEM((S, D), F32),
        pltpu.VMEM((S, D), F32),
        pltpu.VMEM((S + 2 * HPAD, D), F32),
        pltpu.VMEM((G, L, 128), BF16),
        pltpu.VMEM((G, L, 128), BF16),
        pltpu.VMEM((D, L), BF16),
        pltpu.VMEM((D, L), BF16),
        pltpu.VMEM((D, L), BF16),
        pltpu.VMEM((G, L, 128), BF16),
        pltpu.VMEM((G, 128, 128), F32),
        pltpu.VMEM((G, 16, 128), F32),
        pltpu.VMEM((NSEG, L, D), BF16),
        pltpu.SemaphoreType.DMA((NSEG + 8,)),
        pltpu.SemaphoreType.DMA((NSEG,)),
    ]
    out = pl.pallas_call(
        _kernel,
        out_shape=jax.ShapeDtypeStruct((S, D), BF16),
        in_specs=[pl.BlockSpec(memory_space=pltpu.SMEM)] + [any_spec] * 9,
        out_specs=any_spec,
        scratch_shapes=scratch,
        compiler_params=pltpu.CompilerParams(vmem_limit_bytes=120 * 1024 * 1024),
    )(beta, x, A_wq, A_wk, A_wv, A_wo, B_w1, B_w2, B_w3, B_w4)
    return out.reshape(1, S, D)
```

```python
import functools

import jax
import jax.numpy as jnp
from jax import lax
import jax.experimental.pallas as pl
import jax.experimental.pallas.tpu as pltpu

S = 2048
D = 1024
H = 32
DH = 32
NSEG = 4
L = 512
F = 3584
G = 8
HPG = 4
QT = 128
NQT = L // QT
HPAD = 8
FC = 512
RC = L // G
TB = 256
NTB = S // TB
TO = 128

LOG2E = 1.4426950408889634
QSCALE = (DH ** -0.5) * LOG2E
MASK_BIAS = -1000000000.0 * LOG2E
GELU_C = 0.7978845608028654

F32 = jnp.float32
BF16 = jnp.bfloat16

NT = (((1,), (1,)), ((), ()))


def _ln(x):
    m = jnp.mean(x, axis=-1, keepdims=True)
    d = x - m
    v = jnp.mean(d * d, axis=-1, keepdims=True)
    return d * lax.rsqrt(v + 1e-05)


def _gelu(x):
    return 0.5 * x * (1.0 + jnp.tanh(GELU_C * (x + 0.044715 * (x * x * x))))


def _phi(t):
    return jnp.where(t > 0, t + 1.0, jnp.exp(t))


def _dot(a, b):
    return jnp.dot(a, b, preferred_element_type=F32)


def _kernel(beta_ref, x_hbm, wq_hbm, wk_hbm, wv_hbm, wo_hbm, w1_hbm, w2_hbm, w3_hbm, w4_hbm,
            out_hbm,
            xin, wq, wk, wv, wo, w1, w2, w3, w4, wqt, wvt,
            xres, xn, ybuf, hbuf, kb, pkb, qt, pqt, vt, ob, mt, zr, obuf,
            sem_x, sem_g, sem_w, sem_out):

    def x_copy(s):
        return pltpu.make_async_copy(x_hbm.at[pl.ds(s * L, L)], xin.at[pl.ds(s * L, L)], sem_x.at[s])

    def group_copies(g):
        return [pltpu.make_async_copy(src.at[:, pl.ds(g * 128, 128)], dst.at[g], sem_g.at[g])
                for src, dst in ((wk_hbm, wk), (wq_hbm, wq), (wv_hbm, wv))]

    def group_wait(g):
        for dst in (wk, wq, wv):
            pltpu.make_async_copy(dst.at[g], dst.at[g], sem_g.at[g]).wait()

    def x_wait(s):
        blk = xin.at[pl.ds(pl.multiple_of(s * L, L), L)]
        pltpu.make_async_copy(blk, blk, sem_x.at[s]).wait()

    w_pairs = [(wo_hbm, wo), (w1_hbm, w1), (w2_hbm, w2), (w3_hbm, w3), (w4_hbm, w4)]
    w_copies = [pltpu.make_async_copy(src, dst, sem_w.at[i]) for i, (src, dst) in enumerate(w_pairs)]
    cp_wo, cp_w1, cp_w2, cp_w3, cp_w4 = w_copies

    x_copy(0).start()
    for cp in group_copies(0):
        cp.start()
    x_copy(1).start()
    for g in range(1, G):
        for cp in group_copies(g):
            cp.start()
    cp_wo.start()
    cp_w1.start()
    x_copy(2).start()
    x_copy(3).start()
    for cp in (cp_w2, cp_w3, cp_w4):
        cp.start()

    hbuf[0:HPAD, :] = jnp.zeros((HPAD, D), F32)
    hbuf[HPAD + S:HPAD + S + HPAD, :] = jnp.zeros((HPAD, D), F32)

    def ln_rows(layer, r):
        rows = pl.ds(pl.multiple_of(r, RC), RC)
        x = jnp.where(layer == 0, xin[rows, :].astype(F32), xres[rows, :])
        xres[rows, :] = x
        xn[rows, :] = _ln(x).astype(BF16)

    def seg_rows(s):
        return pl.ds(pl.multiple_of(s * L, L), L)

    def proj_k(s, g):
        k = _dot(xn[seg_rows(s), :], wk[g])
        kb[...] = k.astype(BF16)
        pkb[...] = _phi(k).astype(BF16)

    def proj_q(s, w):
        q = lax.dot_general(w, xn[seg_rows(s), :], NT, preferred_element_type=F32)
        qt[...] = (q * QSCALE).astype(BF16)
        pqt[...] = _phi(q).astype(BF16)

    def proj_v(s, w):
        v = lax.dot_general(w, xn[seg_rows(s), :], NT, preferred_element_type=F32)
        vt[...] = v.astype(BF16)

    def transposed(src, dst, g):
        w = src[g].T
        dst[g] = w
        return w

    def out_wo(s, r, n):
        rows = pl.ds(pl.multiple_of(s * L + r, n), n)
        rin = pl.ds(pl.multiple_of(r, n), n)
        o = jnp.concatenate([ob[s % 2, g, rin, :] for g in range(G)], axis=1)
        xm = xres[rows, :] + _dot(o, wo[...])
        xres[rows, :] = xm
        y = _ln(xm)
        ybuf[rows, :] = y
        return _ln(y).astype(BF16)

    def out_w1(s, r, n, yn):
        hbuf[pl.ds(pl.multiple_of(HPAD + s * L + r, HPAD), n), :] = _gelu(_dot(yn, w1[...]))

    def qk(i):
        nk = QT * (i + 1)
        zero_blk = jnp.zeros((DH, QT), BF16)
        cols = []
        for h in range(HPG):
            blocks = [zero_blk] * HPG
            blocks[h] = qt[h * DH:(h + 1) * DH, i * QT:(i + 1) * QT]
            cols.append(jnp.concatenate(blocks, axis=0))
        return _dot(kb[0:nk, :], jnp.concatenate(cols, axis=1))

    def softmax_pv(i, st):
        nk = QT * (i + 1)
        krow = lax.broadcasted_iota(jnp.int32, (QT, QT), 0)
        qcol = lax.broadcasted_iota(jnp.int32, (QT, QT), 1)
        bias = jnp.where(krow > qcol, MASK_BIAS, 0.0).astype(F32)
        res = []
        for h in range(HPG):
            sc = st[:, h * QT:(h + 1) * QT]
            diag = sc[nk - QT:, :] + bias
            sc = diag if i == 0 else jnp.concatenate([sc[:nk - QT, :], diag], axis=0)
            m = jnp.max(sc, axis=0, keepdims=True)
            p = jnp.exp2(sc - m)
            l = jnp.sum(p, axis=0, keepdims=True)
            res.append((_dot(vt[h * DH:(h + 1) * DH, 0:nk], p.astype(BF16)), l))
        return res

    def mem_read(g):
        mem = jnp.concatenate([mt[g], zr[g]], axis=0).astype(BF16)
        return _dot(mem, pqt[...])

    def mem_update(g):
        vaug = jnp.concatenate([vt[...], jnp.ones((16, L), BF16)], axis=0)
        upd = _dot(vaug, pkb[...])
        rh = lax.broadcasted_iota(jnp.int32, (144, 128), 0)
        ch = lax.broadcasted_iota(jnp.int32, (144, 128), 1) // DH
        upd = jnp.where(jnp.where(rh < 128, rh // DH, rh - 128) == ch, upd, 0.0)
        mt[g] = mt[g] + upd[:128]
        zr[g] = zr[g] + upd[128:]

    def combine(s, g, nd, res):
        rows = []
        for h in range(HPG):
            gate = jax.nn.sigmoid(jnp.full((1, L), beta_ref[g * HPG + h], F32))
            l_h = jnp.concatenate([res[i][h][1] for i in range(NQT)], axis=1)
            o_h = jnp.concatenate([res[i][h][0] for i in range(NQT)], axis=1)
            c_dot = (1.0 - gate) / l_h
            c_mem = gate / (nd[128 + h:129 + h, :] + 1e-06)
            rows.append(c_mem * nd[h * DH:(h + 1) * DH, :] + c_dot * o_h)
        ob[s % 2, g] = jnp.concatenate(rows, axis=0).T.astype(BF16)

    def attn_first(layer, g):
        sn = (g + 1) // G
        gn = (g + 1) % G

        @pl.when(jnp.logical_and(layer == 0, g < G - 1))
        def _():
            group_wait(gn)

        ln_rows(layer, L + g * RC)
        res = [None] * NQT
        nd = mem_read(g)
        st = [None] * NQT
        for i in reversed(range(NQT)):
            st[i] = qk(i)
        proj_q(sn, transposed(wq, wqt, gn))
        res[3] = softmax_pv(3, st[3])
        res[2] = softmax_pv(2, st[2])
        mem_update(g)
        proj_k(sn, gn)
        res[1] = softmax_pv(1, st[1])
        res[0] = softmax_pv(0, st[0])
        proj_v(sn, transposed(wv, wvt, gn))
        combine(0, g, nd, res)

    def attn_rest(layer, j):
        s = j // G
        g = j % G
        jn = jnp.minimum(j + 1, NSEG * G - 1)
        sn = jn // G
        gn = jn % G

        @pl.when(jnp.logical_and(layer == 0, jnp.logical_and(g == 0, s < NSEG - 1)))
        def _():
            x_wait(s + 1)

        ln_rows(layer, jnp.minimum(s + 1, NSEG - 1) * L + g * RC)
        res = [None] * NQT
        nd = mem_read(g)
        st3 = qk(3)
        yn = out_wo(s - 1, g * RC, RC)
        st2 = qk(2)
        res[3] = softmax_pv(3, st3)
        mem_update(g)
        st1 = qk(1)
        st0 = qk(0)
        proj_q(sn, wqt[gn])
        res[2] = softmax_pv(2, st2)
        out_w1(s - 1, g * RC, RC, yn)
        res[1] = softmax_pv(1, st1)
        res[0] = softmax_pv(0, st0)
        proj_k(sn, gn)
        proj_v(sn, wvt[gn])
        combine(s, g, nd, res)

    def out_copy(t):
        rows = pl.ds(pl.multiple_of(t * TB, TB), TB)
        return pltpu.make_async_copy(obuf.at[rows], out_hbm.at[rows], sem_out.at[t])

    def b_step(t, layer):
        r = pl.multiple_of(t * TB, TB)
        c = D // 4
        win = hbuf[pl.ds(r, TB + 2 * HPAD), :]
        parts = []
        for ci, off in enumerate((-1, 1, -2, 2)):
            parts.append(win[HPAD + off:HPAD + off + TB, ci * c:(ci + 1) * c].astype(BF16))
        gsh = jnp.concatenate(parts, axis=1)
        x1 = ybuf[pl.ds(r, TB), :] + _dot(gsh, w2[...])
        x1n = _ln(x1).astype(BF16)
        acc = xres[pl.ds(r, TB), :] + x1
        for ci in range(F // FC):
            h = _gelu(_dot(x1n, w3[:, ci * FC:(ci + 1) * FC])).astype(BF16)
            acc = acc + _dot(h, w4[ci * FC:(ci + 1) * FC, :])
        xres[pl.ds(r, TB), :] = acc
        obuf[pl.ds(r, TB), :] = acc.astype(BF16)

        @pl.when(layer == 1)
        def _():
            out_copy(t).start()

    def loop(lo, hi, fn):
        def body(i, c):
            fn(i)
            return c
        lax.fori_loop(lo, hi, body, 0)

    def layer_body(layer):
        mt[...] = jnp.zeros(mt.shape, F32)
        zr[...] = jnp.zeros(zr.shape, F32)

        @pl.when(layer == 0)
        def _():
            x_wait(0)

        loop(0, G, lambda i: ln_rows(layer, i * RC))

        @pl.when(layer == 0)
        def _():
            group_wait(0)

        proj_k(0, 0)
        proj_q(0, transposed(wq, wqt, 0))
        proj_v(0, transposed(wv, wvt, 0))

        @pl.when(layer == 0)
        def _():
            x_wait(1)

        loop(0, G, lambda g: attn_first(layer, g))

        @pl.when(layer == 0)
        def _():
            cp_wo.wait()
            cp_w1.wait()

        loop(G, NSEG * G, lambda j: attn_rest(layer, j))
        loop(0, L // TO, lambda i: out_w1(NSEG - 1, i * TO, TO, out_wo(NSEG - 1, i * TO, TO)))

        @pl.when(layer == 0)
        def _():
            cp_w2.wait()
            cp_w3.wait()
            cp_w4.wait()

        loop(0, NTB, lambda t: b_step(t, layer))

    loop(0, 2, layer_body)

    for t in range(NTB):
        out_copy(t).wait()


@jax.jit
def pallas_interleave_layers__memory_aug_infini_attn__mixer_s_mlp__prompt_kernel(
    A_x: jax.Array,
    A_wq: jax.Array,
    A_wk: jax.Array,
    A_wv: jax.Array,
    A_wo: jax.Array,
    A_beta: jax.Array,
    B_x: jax.Array,
    B_w1: jax.Array,
    B_w2: jax.Array,
    B_w3: jax.Array,
    B_w4: jax.Array,
):
    del B_x
    x = A_x.reshape(S, D)
    beta = A_beta.astype(F32)
    any_spec = pl.BlockSpec(memory_space=pl.ANY)
    scratch = [
        pltpu.VMEM((S, D), BF16),
        pltpu.VMEM((G, D, 128), BF16),
        pltpu.VMEM((G, D, 128), BF16),
        pltpu.VMEM((G, D, 128), BF16),
        pltpu.VMEM((D, D), BF16),
        pltpu.VMEM((D, D), BF16),
        pltpu.VMEM((D, D), BF16),
        pltpu.VMEM((D, F), BF16),
        pltpu.VMEM((F, D), BF16),
        pltpu.VMEM((G, 128, D), BF16),
        pltpu.VMEM((G, 128, D), BF16),
        pltpu.VMEM((S, D), F32),
        pltpu.VMEM((S, D), BF16),
        pltpu.VMEM((S, D), F32),
        pltpu.VMEM((S + 2 * HPAD, D), F32),
        pltpu.VMEM((L, 128), BF16),
        pltpu.VMEM((L, 128), BF16),
        pltpu.VMEM((128, L), BF16),
        pltpu.VMEM((128, L), BF16),
        pltpu.VMEM((128, L), BF16),
        pltpu.VMEM((2, G, L, 128), BF16),
        pltpu.VMEM((G, 128, 128), F32),
        pltpu.VMEM((G, 16, 128), F32),
        pltpu.VMEM((S, D), BF16),
        pltpu.SemaphoreType.DMA((NSEG,)),
        pltpu.SemaphoreType.DMA((G,)),
        pltpu.SemaphoreType.DMA((5,)),
        pltpu.SemaphoreType.DMA((NTB,)),
    ]
    out = pl.pallas_call(
        _kernel,
        out_shape=jax.ShapeDtypeStruct((S, D), BF16),
        in_specs=[pl.BlockSpec(memory_space=pltpu.SMEM)] + [any_spec] * 9,
        out_specs=any_spec,
        scratch_shapes=scratch,
        compiler_params=pltpu.CompilerParams(vmem_limit_bytes=120 * 1024 * 1024),
    )(beta, x, A_wq, A_wk, A_wv, A_wo, B_w1, B_w2, B_w3, B_w4)
    return out.reshape(1, S, D)
```

```python
import jax
import jax.numpy as jnp
from jax import lax
import jax.experimental.pallas as pl
import jax.experimental.pallas.tpu as pltpu

S = 2048
D = 1024
H = 32
DH = 32
NSEG = 4
L = 512
F = 3584
G = 8
HPG = 4
QT = 128
NQT = L // QT
HPAD = 8
FC = 512
RC = L // G
TB = 256
NTB = S // TB
TO = 128

LOG2E = 1.4426950408889634
QSCALE = (DH ** -0.5) * LOG2E
MASK_BIAS = -1000000000.0 * LOG2E
GELU_C = 0.7978845608028654
SAFE_LOGIT = 40.0

F32 = jnp.float32
BF16 = jnp.bfloat16

NT = (((1,), (1,)), ((), ()))
ORDER_FIRST = "ln S0 S1 P0 S2 P1 S3 P2 mr mu q P3 c k v"
ORDER_REST = "ln S0 S1 P0 S2 P1 S3 P2 mr mu q P3 c k wo v w1"


def _ln(x):
    m = jnp.mean(x, axis=-1, keepdims=True)
    d = x - m
    v = jnp.mean(d * d, axis=-1, keepdims=True)
    return d * lax.rsqrt(v + 1e-05)


def _gelu(x):
    return 0.5 * x * (1.0 + jnp.tanh(GELU_C * (x + 0.044715 * (x * x * x))))


def _phi(t):
    return jnp.where(t > 0, t + 1.0, jnp.exp(t))


def _dot(a, b):
    return jnp.dot(a, b, preferred_element_type=F32)


def _kernel(beta_ref, x_hbm, wq_hbm, wk_hbm, wv_hbm, wo_hbm, w1_hbm, w2_hbm, w3_hbm, w4_hbm,
            out_hbm,
            xin, wq, wk, wv, wo, w1, w2, w3, w4, wqt, wvt,
            xres, xn, ybuf, hbuf, kb, pkb, qt, pqt, vt, ob, mt, zr, obuf, shift, amax,
            sem_x, sem_g, sem_w, sem_out):

    def x_copy(s):
        return pltpu.make_async_copy(x_hbm.at[pl.ds(s * L, L)], xin.at[pl.ds(s * L, L)], sem_x.at[s])

    def group_copies(g):
        return [pltpu.make_async_copy(src.at[:, pl.ds(g * 128, 128)], dst.at[g], sem_g.at[g])
                for src, dst in ((wk_hbm, wk), (wq_hbm, wq), (wv_hbm, wv))]

    def group_wait(g):
        for dst in (wk, wq, wv):
            pltpu.make_async_copy(dst.at[g], dst.at[g], sem_g.at[g]).wait()

    def x_wait(s):
        blk = xin.at[pl.ds(pl.multiple_of(s * L, L), L)]
        pltpu.make_async_copy(blk, blk, sem_x.at[s]).wait()

    w_pairs = [(wo_hbm, wo), (w1_hbm, w1), (w2_hbm, w2), (w3_hbm, w3), (w4_hbm, w4)]
    w_copies = [pltpu.make_async_copy(src, dst, sem_w.at[i]) for i, (src, dst) in enumerate(w_pairs)]
    cp_wo, cp_w1, cp_w2, cp_w3, cp_w4 = w_copies

    def start_groups(groups):
        for g in groups:
            for cp in group_copies(g):
                cp.start()

    x_copy(0).start()
    start_groups([0])

    hbuf[0:HPAD, :] = jnp.zeros((HPAD, D), F32)
    hbuf[HPAD + S:HPAD + S + HPAD, :] = jnp.zeros((HPAD, D), F32)

    def residual(layer, rows):
        return jnp.where(layer == 0, xin[rows, :].astype(F32), xres[rows, :])

    def ln_rows(layer, r):
        rows = pl.ds(pl.multiple_of(r, RC), RC)
        xn[rows, :] = _ln(residual(layer, rows)).astype(BF16)

    def seg_rows(s):
        return pl.ds(pl.multiple_of(s * L, L), L)

    def proj_k(s, g):
        k = _dot(xn[seg_rows(s), :], wk[g])
        kb[...] = k.astype(BF16)
        pkb[...] = _phi(k).astype(BF16)
        amax[0] = jnp.max(jnp.abs(k))

    def proj_q(s, w):
        q = lax.dot_general(w, xn[seg_rows(s), :], NT, preferred_element_type=F32)
        qt[...] = (q * QSCALE).astype(BF16)
        pqt[...] = _phi(q).astype(BF16)
        amax[1] = jnp.max(jnp.abs(q))

    def proj_v(s, w):
        v = lax.dot_general(w, xn[seg_rows(s), :], NT, preferred_element_type=F32)
        vt[...] = v.astype(BF16)

    def transposed(src, dst, g):
        w = src[g].T
        dst[g] = w
        return w

    def out_wo(layer, s, r, n):
        rows = pl.ds(pl.multiple_of(s * L + r, n), n)
        rin = pl.ds(pl.multiple_of(r, n), n)
        o = jnp.concatenate([ob[s % 2, g, rin, :] for g in range(G)], axis=1)
        xm = residual(layer, rows) + _dot(o, wo[...])
        xres[rows, :] = xm
        y = _ln(xm)
        ybuf[rows, :] = y
        return _ln(y).astype(BF16)

    def out_w1(s, r, n, yn):
        hbuf[pl.ds(pl.multiple_of(HPAD + s * L + r, HPAD), n), :] = _gelu(_dot(yn, w1[...]))

    def qk(i):
        nk = QT * (i + 1)
        zero_blk = jnp.zeros((DH, QT), BF16)
        cols = []
        for h in range(HPG):
            blocks = [zero_blk] * HPG
            blocks[h] = qt[h * DH:(h + 1) * DH, i * QT:(i + 1) * QT]
            cols.append(jnp.concatenate(blocks, axis=0))
        return _dot(kb[0:nk, :], jnp.concatenate(cols, axis=1))

    def masked(i, st, h):
        nk = QT * (i + 1)
        krow = lax.broadcasted_iota(jnp.int32, (QT, QT), 0)
        qcol = lax.broadcasted_iota(jnp.int32, (QT, QT), 1)
        bias = jnp.where(krow > qcol, MASK_BIAS, 0.0).astype(F32)
        sc = st[:, h * QT:(h + 1) * QT]
        diag = sc[nk - QT:, :] + bias
        return diag if i == 0 else jnp.concatenate([sc[:nk - QT, :], diag], axis=0)

    def softmax_shift():
        bound = amax[0] * amax[1] * (DH * QSCALE * 1.02)
        safe = bound <= SAFE_LOGIT

        @pl.when(safe)
        def _():
            shift[...] = jnp.zeros(shift.shape, F32)

        @pl.when(jnp.logical_not(safe))
        def _():
            for i in range(NQT):
                st = qk(i)
                for h in range(HPG):
                    row = i * HPG + h
                    shift[row:row + 1, :] = jnp.max(masked(i, st, h), axis=0, keepdims=True)

    def probs(i):
        st = qk(i)
        res = []
        for h in range(HPG):
            row = i * HPG + h
            p = jnp.exp2(masked(i, st, h) - shift[row:row + 1, :])
            res.append((p.astype(BF16), jnp.sum(p, axis=0, keepdims=True)))
        return res

    def pv(i, ps):
        nk = QT * (i + 1)
        return [(_dot(vt[h * DH:(h + 1) * DH, 0:nk], ps[h][0]), ps[h][1]) for h in range(HPG)]

    def mem_read(g):
        mem = jnp.concatenate([mt[g], zr[g]], axis=0).astype(BF16)
        return _dot(mem, pqt[...])

    def mem_update(g):
        vaug = jnp.concatenate([vt[...], jnp.ones((16, L), BF16)], axis=0)
        upd = _dot(vaug, pkb[...])
        rh = lax.broadcasted_iota(jnp.int32, (144, 128), 0)
        ch = lax.broadcasted_iota(jnp.int32, (144, 128), 1) // DH
        upd = jnp.where(jnp.where(rh < 128, rh // DH, rh - 128) == ch, upd, 0.0)
        mt[g] = mt[g] + upd[:128]
        zr[g] = zr[g] + upd[128:]

    def combine(s, g, nd, res):
        rows = []
        for h in range(HPG):
            gate = jax.nn.sigmoid(jnp.full((1, L), beta_ref[g * HPG + h], F32))
            l_h = jnp.concatenate([res[i][h][1] for i in range(NQT)], axis=1)
            o_h = jnp.concatenate([res[i][h][0] for i in range(NQT)], axis=1)
            c_dot = (1.0 - gate) / l_h
            c_mem = gate / (nd[128 + h:129 + h, :] + 1e-06)
            rows.append(c_mem * nd[h * DH:(h + 1) * DH, :] + c_dot * o_h)
        ob[s % 2, g] = jnp.concatenate(rows, axis=0).T.astype(BF16)

    def run(layer, order, s, g, sn, gn, get_wq, get_wv):
        ps, res, tmp = {}, {}, {}
        for op in order.split():
            if op[0] == "S":
                ps[int(op[1])] = probs(int(op[1]))
            elif op[0] == "P":
                res[int(op[1])] = pv(int(op[1]), ps[int(op[1])])
            elif op == "mr":
                tmp["nd"] = mem_read(g)
            elif op == "mu":
                mem_update(g)
            elif op == "wo":
                tmp["yn"] = out_wo(layer, s - 1, g * RC, RC)
            elif op == "w1":
                out_w1(s - 1, g * RC, RC, tmp["yn"])
            elif op == "q":
                proj_q(sn, get_wq())
            elif op == "k":
                proj_k(sn, gn)
            elif op == "v":
                proj_v(sn, get_wv())
            elif op == "ln":
                ln_rows(layer, jnp.minimum(s + 1, NSEG - 1) * L + g * RC)
            elif op == "c":
                combine(s, g, tmp["nd"], res)

    def attn_first(layer, g):
        sn = (g + 1) // G
        gn = (g + 1) % G

        @pl.when(jnp.logical_and(layer == 0, g < G - 1))
        def _():
            group_wait(gn)

        @pl.when(jnp.logical_and(layer == 0, g == 2))
        def _():
            cp_wo.start()
            cp_w1.start()
            x_copy(2).start()
            x_copy(3).start()

        softmax_shift()
        run(layer, ORDER_FIRST, 0, g, sn, gn, lambda: transposed(wq, wqt, gn), lambda: transposed(wv, wvt, gn))

    def attn_rest(layer, j):
        s = j // G
        g = j % G
        jn = jnp.minimum(j + 1, NSEG * G - 1)
        sn = jn // G
        gn = jn % G

        @pl.when(jnp.logical_and(layer == 0, jnp.logical_and(g == 0, s < NSEG - 1)))
        def _():
            x_wait(s + 1)

        softmax_shift()
        run(layer, ORDER_REST, s, g, sn, gn, lambda: wqt[gn], lambda: wvt[gn])

    def out_copy(t):
        rows = pl.ds(pl.multiple_of(t * TB, TB), TB)
        return pltpu.make_async_copy(obuf.at[rows], out_hbm.at[rows], sem_out.at[t])

    def b_step(t, layer):
        r = pl.multiple_of(t * TB, TB)
        c = D // 4
        win = hbuf[pl.ds(r, TB + 2 * HPAD), :]
        parts = []
        for ci, off in enumerate((-1, 1, -2, 2)):
            parts.append(win[HPAD + off:HPAD + off + TB, ci * c:(ci + 1) * c].astype(BF16))
        gsh = jnp.concatenate(parts, axis=1)
        x1 = ybuf[pl.ds(r, TB), :] + _dot(gsh, w2[...])
        x1n = _ln(x1).astype(BF16)
        acc = xres[pl.ds(r, TB), :] + x1
        for ci in range(F // FC):
            h = _gelu(_dot(x1n, w3[:, ci * FC:(ci + 1) * FC])).astype(BF16)
            acc = acc + _dot(h, w4[ci * FC:(ci + 1) * FC, :])
        xres[pl.ds(r, TB), :] = acc
        obuf[pl.ds(r, TB), :] = acc.astype(BF16)

        @pl.when(layer == 1)
        def _():
            out_copy(t).start()

    def loop(lo, hi, fn):
        def body(i, c):
            fn(i)
            return c
        lax.fori_loop(lo, hi, body, 0)

    def layer_body(layer):
        mt[...] = jnp.zeros(mt.shape, F32)
        zr[...] = jnp.zeros(zr.shape, F32)

        @pl.when(layer == 0)
        def _():
            x_wait(0)
            x_copy(1).start()
            start_groups([1])

        loop(0, G, lambda i: ln_rows(layer, i * RC))

        @pl.when(layer == 0)
        def _():
            group_wait(0)
            start_groups(range(2, G))

        proj_k(0, 0)
        proj_q(0, transposed(wq, wqt, 0))
        proj_v(0, transposed(wv, wvt, 0))

        @pl.when(layer == 0)
        def _():
            x_wait(1)

        loop(0, G, lambda g: attn_first(layer, g))

        @pl.when(layer == 0)
        def _():
            cp_wo.wait()
            cp_w1.wait()
            for cp in (cp_w2, cp_w3, cp_w4):
                cp.start()

        loop(G, NSEG * G, lambda j: attn_rest(layer, j))
        loop(0, L // TO, lambda i: out_w1(NSEG - 1, i * TO, TO, out_wo(layer, NSEG - 1, i * TO, TO)))

        @pl.when(layer == 0)
        def _():
            cp_w2.wait()
            cp_w3.wait()
            cp_w4.wait()

        loop(0, NTB, lambda t: b_step(t, layer))

    loop(0, 2, layer_body)

    for t in range(NTB):
        out_copy(t).wait()


@jax.jit
def pallas_interleave_layers__memory_aug_infini_attn__mixer_s_mlp__prompt_kernel(
    A_x: jax.Array,
    A_wq: jax.Array,
    A_wk: jax.Array,
    A_wv: jax.Array,
    A_wo: jax.Array,
    A_beta: jax.Array,
    B_x: jax.Array,
    B_w1: jax.Array,
    B_w2: jax.Array,
    B_w3: jax.Array,
    B_w4: jax.Array,
):
    del B_x
    x = A_x.reshape(S, D)
    beta = A_beta.astype(F32)
    any_spec = pl.BlockSpec(memory_space=pl.ANY)
    scratch = [
        pltpu.VMEM((S, D), BF16),
        pltpu.VMEM((G, D, 128), BF16),
        pltpu.VMEM((G, D, 128), BF16),
        pltpu.VMEM((G, D, 128), BF16),
        pltpu.VMEM((D, D), BF16),
        pltpu.VMEM((D, D), BF16),
        pltpu.VMEM((D, D), BF16),
        pltpu.VMEM((D, F), BF16),
        pltpu.VMEM((F, D), BF16),
        pltpu.VMEM((G, 128, D), BF16),
        pltpu.VMEM((G, 128, D), BF16),
        pltpu.VMEM((S, D), F32),
        pltpu.VMEM((S, D), BF16),
        pltpu.VMEM((S, D), F32),
        pltpu.VMEM((S + 2 * HPAD, D), F32),
        pltpu.VMEM((L, 128), BF16),
        pltpu.VMEM((L, 128), BF16),
        pltpu.VMEM((128, L), BF16),
        pltpu.VMEM((128, L), BF16),
        pltpu.VMEM((128, L), BF16),
        pltpu.VMEM((2, G, L, 128), BF16),
        pltpu.VMEM((G, 128, 128), F32),
        pltpu.VMEM((G, 16, 128), F32),
        pltpu.VMEM((S, D), BF16),
        pltpu.VMEM((NQT * HPG, QT), F32),
        pltpu.SMEM((2,), F32),
        pltpu.SemaphoreType.DMA((NSEG,)),
        pltpu.SemaphoreType.DMA((G,)),
        pltpu.SemaphoreType.DMA((5,)),
        pltpu.SemaphoreType.DMA((NTB,)),
    ]
    out = pl.pallas_call(
        _kernel,
        out_shape=jax.ShapeDtypeStruct((S, D), BF16),
        in_specs=[pl.BlockSpec(memory_space=pltpu.SMEM)] + [any_spec] * 9,
        out_specs=any_spec,
        scratch_shapes=scratch,
        compiler_params=pltpu.CompilerParams(vmem_limit_bytes=120 * 1024 * 1024),
    )(beta, x, A_wq, A_wk, A_wv, A_wo, B_w1, B_w2, B_w3, B_w4)
    return out.reshape(1, S, D)
```

```python
import functools

import jax
import jax.numpy as jnp
from jax import lax
import jax.experimental.pallas as pl
import jax.experimental.pallas.tpu as pltpu

S = 2048
D = 1024
H = 32
DH = 32
NSEG = 4
L = 512
F = 3584
G = 8
HPG = 4
QT = 128
NQT = L // QT
HPAD = 8
FC = 512
RC = L // G
TB = 256
NTB = S // TB
NHALF = 2
TO = 256

LOG2E = 1.4426950408889634
QSCALE = (DH ** -0.5) * LOG2E
MASK_BIAS = -1000000000.0 * LOG2E
GELU_C = 0.7978845608028654
SAFE_LOGIT = 40.0

F32 = jnp.float32
BF16 = jnp.bfloat16

NT = (((1,), (1,)), ((), ()))
SHIFTS = (-1, 1, -2, 2)
ORDER_FIRST = "ln S0 S1 P0 S2 P1 S3 P2 mr mu q P3 c k v"
ORDER_LAST = "S3 wo S2 P3 S1 P2 S0 mr P1 P0 c w1"
ORDER_REST = "ln S0 S1 P0 S2 P1 S3 P2 mr mu q P3 c k wo v w1"


def _ln(x):
    m = jnp.mean(x, axis=-1, keepdims=True)
    d = x - m
    v = jnp.mean(d * d, axis=-1, keepdims=True)
    return d * lax.rsqrt(v + 1e-05)


def _gelu(x):
    return 0.5 * x * (1.0 + jnp.tanh(GELU_C * (x + 0.044715 * (x * x * x))))


def _phi(t):
    return jnp.where(t > 0, t + 1.0, jnp.exp(t))


def _dot(a, b):
    return jnp.dot(a, b, preferred_element_type=F32)


def _kernel(beta_ref, x_hbm, wq_hbm, wk_hbm, wv_hbm, wo_hbm, w1_hbm, w2_hbm, w3_hbm, w4_hbm,
            out_hbm,
            xin, wq, wk, wv, wo, w1, w2, w3, w4, wqt, wvt,
            xres, xn, ybuf, hbuf, kb, pkb, qt, pqt, vt, ob, mt, zr, obuf, shift, amax,
            sem_x, sem_g, sem_w, sem_out):

    def x_copy(s):
        return pltpu.make_async_copy(x_hbm.at[pl.ds(s * L, L)], xin.at[pl.ds(s * L, L)], sem_x.at[s])

    def group_copies(g):
        return [pltpu.make_async_copy(src.at[:, pl.ds(g * 128, 128)], dst.at[g], sem_g.at[g])
                for src, dst in ((wk_hbm, wk), (wq_hbm, wq), (wv_hbm, wv))]

    def group_wait(g):
        for dst in (wk, wq, wv):
            pltpu.make_async_copy(dst.at[g], dst.at[g], sem_g.at[g]).wait()

    def x_wait(s):
        blk = xin.at[pl.ds(s * L, L)]
        pltpu.make_async_copy(blk, blk, sem_x.at[s]).wait()

    w_pairs = [(wo_hbm, wo), (w1_hbm, w1), (w2_hbm, w2), (w3_hbm, w3), (w4_hbm, w4)]
    w_copies = [pltpu.make_async_copy(src, dst, sem_w.at[i]) for i, (src, dst) in enumerate(w_pairs)]
    cp_wo, cp_w1, cp_w2, cp_w3, cp_w4 = w_copies

    def start_groups(groups):
        for g in groups:
            for cp in group_copies(g):
                cp.start()

    x_copy(0).start()
    start_groups([0])

    hbuf[:, 0:HPAD, :] = jnp.zeros((D // 128, HPAD, 128), F32)
    hbuf[:, HPAD + S:HPAD + S + HPAD, :] = jnp.zeros((D // 128, HPAD, 128), F32)

    def residual(layer, rows):
        return jnp.where(layer == 0, xin[rows, :].astype(F32), xres[rows, :])

    def ln_rows(layer, r, n=RC):
        rows = pl.ds(pl.multiple_of(r, n), n)
        xn[rows, :] = _ln(residual(layer, rows)).astype(BF16)

    def seg_rows(s):
        return pl.ds(pl.multiple_of(s * L, L), L)

    def proj_k(s, g):
        k = _dot(xn[seg_rows(s), :], wk[g])
        kb[...] = k.astype(BF16)
        pkb[...] = _phi(k).astype(BF16)
        amax[0] = jnp.max(jnp.abs(k))

    def proj_q(s, w):
        q = lax.dot_general(w, xn[seg_rows(s), :], NT, preferred_element_type=F32)
        qt[...] = (q * QSCALE).astype(BF16)
        pqt[...] = _phi(q).astype(BF16)
        amax[1] = jnp.max(jnp.abs(q))

    def proj_v(s, w):
        v = lax.dot_general(w, xn[seg_rows(s), :], NT, preferred_element_type=F32)
        vt[...] = v.astype(BF16)

    def transposed(src, dst, g):
        w = src[g].T
        dst[g] = w
        return w

    def layer_head(layer):
        wqg = transposed(wq, wqt, 0)
        wvg = transposed(wv, wvt, 0)
        kmax, qmax = [], []
        for c in range(L // QT):
            rows = pl.ds(c * QT, QT)
            xc = _ln(residual(layer, rows)).astype(BF16)
            xn[rows, :] = xc
            k = _dot(xc, wk[0])
            kb[rows, :] = k.astype(BF16)
            pkb[rows, :] = _phi(k).astype(BF16)
            kmax.append(jnp.abs(k))
            q = lax.dot_general(wqg, xc, NT, preferred_element_type=F32)
            qt[:, rows] = (q * QSCALE).astype(BF16)
            pqt[:, rows] = _phi(q).astype(BF16)
            qmax.append(jnp.abs(q))
            vt[:, rows] = lax.dot_general(wvg, xc, NT, preferred_element_type=F32).astype(BF16)
        amax[0] = jnp.max(functools.reduce(jnp.maximum, kmax))
        amax[1] = jnp.max(functools.reduce(jnp.maximum, qmax))

    def out_wo(layer, s, r, n):
        rows = pl.ds(pl.multiple_of(s * L + r, n), n)
        rin = pl.ds(pl.multiple_of(r, n), n)
        o = jnp.concatenate([ob[s & 1, g, rin, :] for g in range(G)], axis=1)
        xm = residual(layer, rows) + _dot(o, wo[...])
        xres[rows, :] = xm
        y = _ln(xm)
        ybuf[rows, :] = y
        return _ln(y).astype(BF16)

    def out_w1(s, r, n, yn):
        h = _gelu(_dot(yn, w1[...]))
        rows = pl.ds(pl.multiple_of(HPAD + s * L + r, HPAD), n)
        for cb in range(D // 128):
            hbuf[cb, rows, :] = h[:, cb * 128:(cb + 1) * 128]

    def qk(i):
        nk = QT * (i + 1)
        zero_blk = jnp.zeros((DH, QT), BF16)
        cols = []
        for h in range(HPG):
            blocks = [zero_blk] * HPG
            blocks[h] = qt[h * DH:(h + 1) * DH, i * QT:(i + 1) * QT]
            cols.append(jnp.concatenate(blocks, axis=0))
        return _dot(kb[0:nk, :], jnp.concatenate(cols, axis=1))

    def masked(i, st, h):
        nk = QT * (i + 1)
        krow = lax.broadcasted_iota(jnp.int32, (QT, QT), 0)
        qcol = lax.broadcasted_iota(jnp.int32, (QT, QT), 1)
        bias = jnp.where(krow > qcol, MASK_BIAS, 0.0).astype(F32)
        sc = st[:, h * QT:(h + 1) * QT]
        diag = sc[nk - QT:, :] + bias
        return diag if i == 0 else jnp.concatenate([sc[:nk - QT, :], diag], axis=0)

    def softmax_shift():
        bound = amax[0] * amax[1] * (DH * QSCALE * 1.02)
        safe = bound <= SAFE_LOGIT

        @pl.when(safe)
        def _():
            shift[...] = jnp.zeros(shift.shape, F32)

        @pl.when(jnp.logical_not(safe))
        def _():
            for i in range(NQT):
                st = qk(i)
                for h in range(HPG):
                    row = i * HPG + h
                    shift[row:row + 1, :] = jnp.max(masked(i, st, h), axis=0, keepdims=True)

    def probs(i):
        st = qk(i)
        res = []
        for h in range(HPG):
            row = i * HPG + h
            p = jnp.exp2(masked(i, st, h) - shift[row:row + 1, :])
            res.append((p.astype(BF16), jnp.sum(p, axis=0, keepdims=True)))
        return res

    def pv(i, ps):
        nk = QT * (i + 1)
        return [(_dot(vt[h * DH:(h + 1) * DH, 0:nk], ps[h][0]), ps[h][1]) for h in range(HPG)]

    def mem_read(g):
        mem = jnp.concatenate([mt[g], zr[g]], axis=0).astype(BF16)
        return _dot(mem, pqt[...])

    def mem_update(g):
        vaug = jnp.concatenate([vt[...], jnp.ones((16, L), BF16)], axis=0)
        upd = _dot(vaug, pkb[...])
        rh = lax.broadcasted_iota(jnp.int32, (144, 128), 0)
        ch = lax.broadcasted_iota(jnp.int32, (144, 128), 1) // DH
        upd = jnp.where(jnp.where(rh < 128, rh // DH, rh - 128) == ch, upd, 0.0)
        mt[g] = mt[g] + upd[:128]
        zr[g] = zr[g] + upd[128:]

    def combine(s, g, nd, res):
        rows = []
        for h in range(HPG):
            gate = jax.nn.sigmoid(jnp.full((1, L), beta_ref[g * HPG + h], F32))
            l_h = jnp.concatenate([res[i][h][1] for i in range(NQT)], axis=1)
            o_h = jnp.concatenate([res[i][h][0] for i in range(NQT)], axis=1)
            c_dot = (1.0 - gate) / l_h
            c_mem = gate / (nd[128 + h:129 + h, :] + 1e-06)
            rows.append(c_mem * nd[h * DH:(h + 1) * DH, :] + c_dot * o_h)
        ob[s & 1, g] = jnp.concatenate(rows, axis=0).T.astype(BF16)

    def run(layer, order, s, g, sn, gn, get_wq, get_wv):
        ps, res, tmp = {}, {}, {}
        for op in order.split():
            if op[0] == "S":
                ps[int(op[1])] = probs(int(op[1]))
            elif op[0] == "P":
                res[int(op[1])] = pv(int(op[1]), ps[int(op[1])])
            elif op == "mr":
                tmp["nd"] = mem_read(g)
            elif op == "mu":
                mem_update(g)
            elif op == "wo":
                tmp["yn"] = out_wo(layer, s - 1, g * RC, RC)
            elif op == "w1":
                out_w1(s - 1, g * RC, RC, tmp["yn"])
            elif op == "q":
                proj_q(sn, get_wq())
            elif op == "k":
                proj_k(sn, gn)
            elif op == "v":
                proj_v(sn, get_wv())
            elif op == "ln":
                ln_rows(layer, jnp.minimum(s + 1, NSEG - 1) * L + g * RC)
            elif op == "c":
                combine(s, g, tmp["nd"], res)

    def attn_step(layer, j):
        s = lax.shift_right_logical(j, 3)
        g = j & (G - 1)
        sn = lax.shift_right_logical(j + 1, 3)
        gn = (j + 1) & (G - 1)

        softmax_shift()

        @pl.when(j < G)
        def _():
            run(layer, ORDER_FIRST, 0, g, sn, gn,
                lambda: transposed(wq, wqt, gn), lambda: transposed(wv, wvt, gn))

        @pl.when(jnp.logical_and(j >= G, j < NSEG * G - 1))
        def _():
            run(layer, ORDER_REST, s, g, sn, gn, lambda: wqt[gn], lambda: wvt[gn])

        @pl.when(j == NSEG * G - 1)
        def _():
            run(layer, ORDER_LAST, NSEG - 1, G - 1, None, None, None, None)

    def out_tail(layer, i):
        n = TO // 2
        yns = [out_wo(layer, NSEG - 1, i * TO + u * n, n) for u in range(2)]
        for u in range(2):
            out_w1(NSEG - 1, i * TO + u * n, n, yns[u])

    def out_copy(t):
        rows = pl.ds(pl.multiple_of(t * TB, TB), TB)
        return pltpu.make_async_copy(obuf.at[rows], out_hbm.at[rows], sem_out.at[t])

    def b_step(t, layer):
        r = pl.multiple_of(t * TB, TB)
        hb = TB // NHALF
        x1s, x1ns = [], []
        for u in range(NHALF):
            ru = pl.multiple_of(r + u * hb, hb)
            parts = [hbuf[cb, pl.ds(ru + HPAD + SHIFTS[cb // 2], hb), :] for cb in range(D // 128)]
            x1 = ybuf[pl.ds(ru, hb), :] + _dot(jnp.concatenate(parts, axis=1).astype(BF16), w2[...])
            x1ns.append(_ln(x1))
            x1s.append(xres[pl.ds(ru, hb), :] + x1)
        acc = jnp.concatenate(x1s, axis=0)
        x1n = jnp.concatenate(x1ns, axis=0).astype(BF16)
        for ci in range(F // FC):
            w3c = w3[:, ci * FC:(ci + 1) * FC]
            if ci == 0:
                h = jnp.concatenate([_gelu(_dot(part.astype(BF16), w3c)) for part in x1ns], axis=0).astype(BF16)
            else:
                h = _gelu(_dot(x1n, w3c)).astype(BF16)
            acc = acc + _dot(h, w4[ci * FC:(ci + 1) * FC, :])
        xres[pl.ds(r, TB), :] = acc
        obuf[pl.ds(r, TB), :] = acc.astype(BF16)

        @pl.when(layer == 1)
        def _():
            out_copy(t).start()

    def loop(lo, hi, fn):
        def body(i, c):
            fn(i)
            return c
        lax.fori_loop(lo, hi, body, 0)

    def attn_phase(layer, p):
        @pl.when(jnp.logical_and(layer == 0, p == 0))
        def _():
            x_wait(1)
            group_wait(1)
            start_groups([2, 3, 4])

        @pl.when(jnp.logical_and(layer == 0, p == 1))
        def _():
            for g in (2, 3, 4):
                group_wait(g)
            start_groups([5, 6, 7])

        @pl.when(jnp.logical_and(layer == 0, p == 2))
        def _():
            for g in (5, 6, 7):
                group_wait(g)
            cp_wo.start()
            cp_w1.start()
            x_copy(2).start()
            x_copy(3).start()

        @pl.when(jnp.logical_and(layer == 0, p == 3))
        def _():
            cp_wo.wait()
            cp_w1.wait()
            x_wait(2)
            x_wait(3)
            for cp in (cp_w2, cp_w3, cp_w4):
                cp.start()

        lo = jnp.where(p == 3, G, p)
        hi = jnp.where(p == 3, NSEG * G, jnp.where(p == 2, G, p + 1))
        loop(lo, hi, lambda j: attn_step(layer, j))

    def layer_body(layer):
        mt[...] = jnp.zeros(mt.shape, F32)
        zr[...] = jnp.zeros(zr.shape, F32)

        @pl.when(layer == 0)
        def _():
            x_wait(0)
            group_wait(0)
            x_copy(1).start()
            start_groups([1])

        layer_head(layer)

        loop(0, 4, lambda p: attn_phase(layer, p))
        loop(0, L // TO, lambda i: out_tail(layer, i))

        @pl.when(layer == 0)
        def _():
            cp_w2.wait()
            cp_w3.wait()
            cp_w4.wait()

        loop(0, NTB, lambda t: b_step(t, layer))

    loop(0, 2, layer_body)

    for t in range(NTB):
        out_copy(t).wait()


@jax.jit
def pallas_interleave_layers__memory_aug_infini_attn__mixer_s_mlp__prompt_kernel(
    A_x: jax.Array,
    A_wq: jax.Array,
    A_wk: jax.Array,
    A_wv: jax.Array,
    A_wo: jax.Array,
    A_beta: jax.Array,
    B_x: jax.Array,
    B_w1: jax.Array,
    B_w2: jax.Array,
    B_w3: jax.Array,
    B_w4: jax.Array,
):
    del B_x
    x = A_x.reshape(S, D)
    beta = A_beta.astype(F32)
    any_spec = pl.BlockSpec(memory_space=pl.ANY)
    scratch = [
        pltpu.VMEM((S, D), BF16),
        pltpu.VMEM((G, D, 128), BF16),
        pltpu.VMEM((G, D, 128), BF16),
        pltpu.VMEM((G, D, 128), BF16),
        pltpu.VMEM((D, D), BF16),
        pltpu.VMEM((D, D), BF16),
        pltpu.VMEM((D, D), BF16),
        pltpu.VMEM((D, F), BF16),
        pltpu.VMEM((F, D), BF16),
        pltpu.VMEM((G, 128, D), BF16),
        pltpu.VMEM((G, 128, D), BF16),
        pltpu.VMEM((S, D), F32),
        pltpu.VMEM((S, D), BF16),
        pltpu.VMEM((S, D), F32),
        pltpu.VMEM((D // 128, S + 2 * HPAD, 128), F32),
        pltpu.VMEM((L, 128), BF16),
        pltpu.VMEM((L, 128), BF16),
        pltpu.VMEM((128, L), BF16),
        pltpu.VMEM((128, L), BF16),
        pltpu.VMEM((128, L), BF16),
        pltpu.VMEM((2, G, L, 128), BF16),
        pltpu.VMEM((G, 128, 128), F32),
        pltpu.VMEM((G, 16, 128), F32),
        pltpu.VMEM((S, D), BF16),
        pltpu.VMEM((NQT * HPG, QT), F32),
        pltpu.SMEM((2,), F32),
        pltpu.SemaphoreType.DMA((NSEG,)),
        pltpu.SemaphoreType.DMA((G,)),
        pltpu.SemaphoreType.DMA((5,)),
        pltpu.SemaphoreType.DMA((NTB,)),
    ]
    out = pl.pallas_call(
        _kernel,
        out_shape=jax.ShapeDtypeStruct((S, D), BF16),
        in_specs=[pl.BlockSpec(memory_space=pltpu.SMEM)] + [any_spec] * 9,
        out_specs=any_spec,
        scratch_shapes=scratch,
        compiler_params=pltpu.CompilerParams(vmem_limit_bytes=120 * 1024 * 1024),
    )(beta, x, A_wq, A_wk, A_wv, A_wo, B_w1, B_w2, B_w3, B_w4)
    return out.reshape(1, S, D)
```

```python
import functools

import jax
import jax.numpy as jnp
from jax import lax
import jax.experimental.pallas as pl
import jax.experimental.pallas.tpu as pltpu

S = 2048
D = 1024
H = 32
DH = 32
NSEG = 4
L = 512
F = 3584
G = 8
HPG = 4
QT = 128
NQT = L // QT
HPAD = 8
FC = 512
RC = L // G
NPAIR = (NSEG * G - G - 2) // 2
TB = 256
NTB = S // TB
NHALF = 2
TO = 256

NTO = 2
LOG2E = 1.4426950408889634
QSCALE = (DH ** -0.5) * LOG2E
MASK_BIAS = -1000000000.0 * LOG2E
GELU_C = 0.7978845608028654
SAFE_LOGIT = 40.0

F32 = jnp.float32
BF16 = jnp.bfloat16

NT = (((1,), (1,)), ((), ()))
SHIFTS = (-1, 1, -2, 2)
ORDER_FIRST = "cp S0 S1 P0 S2 P1 S3 P2 mr mu q P3 c k L01 v"
ORDER_LAST = "S3 wo S2 P3 S1 P2 S0 mr P1 P0 c w1"
ORDER_PAIR = "cp S0 S1 P0 S2 P1 S3 P2 mr mu q P3 c k L01 wo v +S0 +S1 +P0 +S2 +P1 +S3 +P2 +mr +mu +q +P3 +c +k w1 +v"


def _ln(x):
    m = jnp.mean(x, axis=-1, keepdims=True)
    d = x - m
    v = jnp.mean(d * d, axis=-1, keepdims=True)
    return d * lax.rsqrt(v + 1e-05)


def _gelu(x):
    return 0.5 * x * (1.0 + jnp.tanh(GELU_C * (x + 0.044715 * (x * x * x))))


def _phi(t):
    return jnp.where(t > 0, t + 1.0, jnp.exp(t))


def _dot(a, b):
    return jnp.dot(a, b, preferred_element_type=F32)


def _kernel(beta_ref, x_hbm, wq_hbm, wk_hbm, wv_hbm, wo_hbm, w1_hbm, w2_hbm, w3_hbm, w4_hbm,
            out_hbm,
            xin, wq, wk, wv, wo, w1, w2, w3, w4, wqt, wvt,
            xres, xmid, xn, ybuf, hbuf, kb, pkb, qt, pqt, vt, ob, mt, zr, obuf, shift, ynb, lnb, amax,
            sem_x, sem_g, sem_w, sem_out):

    def x_copy(s):
        return pltpu.make_async_copy(x_hbm.at[pl.ds(s * L, L)], xin.at[pl.ds(s * L, L)], sem_x.at[s])

    def group_copies(g):
        return [pltpu.make_async_copy(src.at[:, pl.ds(g * 128, 128)], dst.at[g], sem_g.at[g])
                for src, dst in ((wk_hbm, wk), (wq_hbm, wq), (wv_hbm, wv))]

    def group_wait(g):
        for dst in (wk, wq, wv):
            pltpu.make_async_copy(dst.at[g], dst.at[g], sem_g.at[g]).wait()

    def x_wait(s):
        blk = xin.at[pl.ds(s * L, L)]
        pltpu.make_async_copy(blk, blk, sem_x.at[s]).wait()

    w_pairs = [(wo_hbm, wo), (w1_hbm, w1), (w2_hbm, w2), (w3_hbm, w3), (w4_hbm, w4)]
    w_copies = [pltpu.make_async_copy(src, dst, sem_w.at[i]) for i, (src, dst) in enumerate(w_pairs)]
    cp_wo, cp_w1, cp_w2, cp_w3, cp_w4 = w_copies

    def start_groups(groups):
        for g in groups:
            for cp in group_copies(g):
                cp.start()

    x_copy(0).start()
    start_groups([0])

    hbuf[:, 0:HPAD, :] = jnp.zeros((D // 128, HPAD, 128), F32)
    hbuf[:, HPAD + S:HPAD + S + HPAD, :] = jnp.zeros((D // 128, HPAD, 128), F32)

    def loop(lo, hi, fn):
        def body(i, c):
            fn(i)
            return c
        lax.fori_loop(lo, hi, body, 0)

    def residual(layer, rows):
        return jnp.where(layer == 0, xin[rows, :].astype(F32), xres[rows, :])

    def ln_rows(layer, r, n=RC):
        rows = pl.ds(pl.multiple_of(r, n), n)
        xn[rows, :] = _ln(residual(layer, rows)).astype(BF16)

    def seg_rows(s):
        return pl.ds(pl.multiple_of(s * L, L), L)

    def proj_k(b, s, g):
        k = _dot(xn[seg_rows(s), :], wk[g])
        kb[b] = k.astype(BF16)
        pkb[b] = _phi(k).astype(BF16)
        amax[2 * b] = jnp.max(jnp.abs(k))

    def proj_q(b, s, w):
        q = lax.dot_general(w, xn[seg_rows(s), :], NT, preferred_element_type=F32)
        qt[b] = (q * QSCALE).astype(BF16)
        pqt[b] = _phi(q).astype(BF16)
        amax[2 * b + 1] = jnp.max(jnp.abs(q))

    def proj_v(b, s, w):
        v = lax.dot_general(w, xn[seg_rows(s), :], NT, preferred_element_type=F32)
        vt[b] = v.astype(BF16)

    def transposed(src, dst, g):
        w = src[g].T
        dst[g] = w
        return w

    def layer_head(layer, b):
        @pl.when(jnp.logical_and(layer == 0, b == 0))
        def _():
            x_wait(0)
            group_wait(0)
            x_copy(1).start()
            start_groups([1])

        @pl.when(jnp.logical_and(layer == 0, b == 1))
        def _():
            x_wait(1)
            group_wait(1)
            start_groups([2, 3])

        wqg = transposed(wq, wqt, b)
        wvg = transposed(wv, wvt, b)
        kmax, qmax = [], []
        for c in range(L // QT):
            rows = pl.ds(c * QT, QT)
            xc = _ln(residual(layer, rows)).astype(BF16)
            xn[rows, :] = xc
            k = _dot(xc, wk[b])
            kb[b, rows, :] = k.astype(BF16)
            pkb[b, rows, :] = _phi(k).astype(BF16)
            kmax.append(jnp.abs(k))
            q = lax.dot_general(wqg, xc, NT, preferred_element_type=F32)
            qt[b, :, rows] = (q * QSCALE).astype(BF16)
            pqt[b, :, rows] = _phi(q).astype(BF16)
            qmax.append(jnp.abs(q))
            vt[b, :, rows] = lax.dot_general(wvg, xc, NT, preferred_element_type=F32).astype(BF16)
        amax[2 * b] = jnp.max(functools.reduce(jnp.maximum, kmax))
        amax[2 * b + 1] = jnp.max(functools.reduce(jnp.maximum, qmax))
        rows = pl.ds(pl.multiple_of(L + (b - 1) * 2 * RC, 2 * RC), 2 * RC)
        xc = _ln(residual(layer, rows)).astype(BF16)
        xn[rows, :] = xc
        lnb[...] = xc

    def out_wo(layer, s, r, n):
        rows = pl.ds(pl.multiple_of(s * L + r, n), n)
        rin = pl.ds(pl.multiple_of(r, n), n)
        o = jnp.concatenate([ob[s & 1, g, rin, :] for g in range(G)], axis=1)
        xm = residual(layer, rows) + _dot(o, wo[...])
        xmid[rows, :] = xm
        y = _ln(xm)
        ybuf[rows, :] = y
        return _ln(y).astype(BF16)

    def out_proj(layer, s, r, n):
        rows = pl.ds(pl.multiple_of(s * L + r, n), n)
        rin = pl.ds(pl.multiple_of(r, n), n)
        o = jnp.concatenate([ob[s & 1, g, rin, :] for g in range(G)], axis=1)
        xmid[rows, :] = residual(layer, rows) + _dot(o, wo[...])

    def out_norm(s, r, off, m):
        rows = pl.ds(pl.multiple_of(s * L + r + off, m), m)
        y = _ln(xmid[rows, :])
        ybuf[rows, :] = y
        ynb[off:off + m, :] = _ln(y).astype(BF16)

    def out_w1(s, r, n, yn):
        h = _gelu(_dot(yn, w1[...]))
        rows = pl.ds(pl.multiple_of(HPAD + s * L + r, HPAD), n)
        for cb in range(D // 128):
            hbuf[cb, rows, :] = h[:, cb * 128:(cb + 1) * 128]

    def q_cols(b, queries):
        zero_blk = jnp.zeros((DH, QT), BF16)
        cols = []
        for h in range(HPG):
            blocks = [zero_blk] * HPG
            blocks[h] = qt[b, h * DH:(h + 1) * DH, queries]
            cols.append(jnp.concatenate(blocks, axis=0))
        return jnp.concatenate(cols, axis=1)

    def qk(b, i):
        return _dot(kb[b, 0:QT * (i + 1), :], q_cols(b, pl.ds(i * QT, QT)))

    def masked(i, st, h):
        nk = QT * (i + 1)
        krow = lax.broadcasted_iota(jnp.int32, (QT, QT), 0)
        qcol = lax.broadcasted_iota(jnp.int32, (QT, QT), 1)
        bias = jnp.where(krow > qcol, MASK_BIAS, 0.0).astype(F32)
        sc = st[:, h * QT:(h + 1) * QT]
        diag = sc[nk - QT:, :] + bias
        return diag if i == 0 else jnp.concatenate([sc[:nk - QT, :], diag], axis=0)

    def softmax_shift():
        scale = DH * QSCALE * 1.02
        safe = jnp.logical_and(amax[0] * amax[1] * scale <= SAFE_LOGIT,
                               amax[2] * amax[3] * scale <= SAFE_LOGIT)

        @pl.when(safe)
        def _():
            shift[...] = jnp.zeros(shift.shape, F32)

        @pl.when(jnp.logical_not(safe))
        def _():
            def row_max(t):
                b = lax.shift_right_logical(t, 2)
                i = t & (NQT - 1)
                q0 = pl.multiple_of(i * QT, QT)
                st = _dot(kb[b], q_cols(b, pl.ds(q0, QT)))
                krow = lax.broadcasted_iota(jnp.int32, (L, QT), 0)
                qcol = lax.broadcasted_iota(jnp.int32, (L, QT), 1) + q0
                bias = jnp.where(krow > qcol, MASK_BIAS, 0.0).astype(F32)
                for h in range(HPG):
                    sc = st[:, h * QT:(h + 1) * QT] + bias
                    shift[b, pl.ds(i * HPG + h, 1), :] = jnp.max(sc, axis=0, keepdims=True)
            loop(0, 2 * NQT, row_max)

    def probs(b, i):
        st = qk(b, i)
        res = []
        for h in range(HPG):
            row = i * HPG + h
            p = jnp.exp2(masked(i, st, h) - shift[b, row:row + 1, :])
            res.append((p.astype(BF16), jnp.sum(p, axis=0, keepdims=True)))
        return res

    def pv(b, i, ps):
        nk = QT * (i + 1)
        return [(_dot(vt[b, h * DH:(h + 1) * DH, 0:nk], ps[h][0]), ps[h][1]) for h in range(HPG)]

    def mem_read(b, g):
        mem = jnp.concatenate([mt[g], zr[g]], axis=0).astype(BF16)
        return _dot(mem, pqt[b])

    def mem_update(b, g):
        vaug = jnp.concatenate([vt[b], jnp.ones((16, L), BF16)], axis=0)
        upd = _dot(vaug, pkb[b])
        rh = lax.broadcasted_iota(jnp.int32, (144, 128), 0)
        ch = lax.broadcasted_iota(jnp.int32, (144, 128), 1) // DH
        upd = jnp.where(jnp.where(rh < 128, rh // DH, rh - 128) == ch, upd, 0.0)
        mt[g] = mt[g] + upd[:128]
        zr[g] = zr[g] + upd[128:]

    def combine(s, g, nd, res):
        rows = []
        for h in range(HPG):
            gate = jax.nn.sigmoid(jnp.full((1, L), beta_ref[g * HPG + h], F32))
            l_h = jnp.concatenate([res[i][h][1] for i in range(NQT)], axis=1)
            o_h = jnp.concatenate([res[i][h][0] for i in range(NQT)], axis=1)
            c_dot = (1.0 - gate) / l_h
            c_mem = gate / (nd[128 + h:129 + h, :] + 1e-06)
            rows.append(c_mem * nd[h * DH:(h + 1) * DH, :] + c_dot * o_h)
        ob[s & 1, g] = jnp.concatenate(rows, axis=0).T.astype(BF16)

    def run(layer, order, j, slots, cp_row, ln_row, fresh):
        n = RC * len(slots)
        s = lax.shift_right_logical(j, 3)
        state = [({}, {}, {}) for _ in slots]
        shared = {}
        for op in order.split():
            u = op.count("+")
            op = op.lstrip("+")
            b = slots[u]
            ps, res, tmp = state[u]
            g = (j + u) & (G - 1)
            sn = lax.shift_right_logical(j + u + 2, 3)
            gn = (j + u + 2) & (G - 1)
            if op[0] == "S":
                ps[int(op[1])] = probs(b, int(op[1]))
            elif op[0] == "P":
                res[int(op[1])] = pv(b, int(op[1]), ps[int(op[1])])
            elif op == "mr":
                tmp["nd"] = mem_read(b, g)
            elif op == "mu":
                mem_update(b, g)
            elif op == "wo":
                shared["yn"] = out_wo(layer, s - 1, g * RC, n)
            elif op == "w1":
                out_w1(s - 1, g * RC, n, shared["yn"])
            elif op == "q":
                proj_q(b, sn, transposed(wq, wqt, gn) if fresh else wqt[gn])
            elif op == "k":
                proj_k(b, sn, gn)
            elif op == "v":
                proj_v(b, sn, transposed(wv, wvt, gn) if fresh else wvt[gn])
            elif op == "ln":
                ln_rows(layer, ln_row, n)
            elif op[0] == "l":
                m = n // int(op[2])
                ln_rows(layer, ln_row + int(op[1]) * m, m)
            elif op[0] == "L":
                m = n // int(op[2])
                off = int(op[1]) * m
                rows = pl.ds(pl.multiple_of(ln_row + off, m), m)
                dst = pl.ds(pl.multiple_of((ln_row & RC) + off, m), m) if n == RC else pl.ds(off, m)
                lnb[dst, :] = _ln(residual(layer, rows)).astype(BF16)
            elif op == "cp":
                src = pl.ds(pl.multiple_of(cp_row & RC, RC), RC) if n == RC else pl.ds(0, n)
                xn[pl.ds(pl.multiple_of(cp_row, n), n), :] = lnb[src, :]
            elif op == "W":
                out_proj(layer, s - 1, g * RC, n)
            elif op[0] == "y":
                m = n // int(op[2])
                out_norm(s - 1, g * RC, int(op[1]) * m, m)
            elif op == "X":
                out_w1(s - 1, g * RC, n, ynb[0:n, :])
            elif op == "c":
                combine(s, g, tmp["nd"], res)

    def attn_step(layer, it):
        softmax_shift()

        @pl.when(it < G)
        def _():
            run(layer, ORDER_FIRST, it, [it & 1], (it + G + 1) * RC, (it + G + 2) * RC, True)

        @pl.when(jnp.logical_and(it >= G, it < G + NPAIR))
        def _():
            j = pl.multiple_of(2 * it - G, 2)
            run(layer, ORDER_PAIR, j, [0, 1], jnp.minimum(j + G, NSEG * G - 2) * RC,
                jnp.minimum(j + G + 2, NSEG * G - 2) * RC, False)

        @pl.when(it >= G + NPAIR)
        def _():
            j = it + NPAIR
            run(layer, ORDER_LAST, j, [j & 1], None, None, False)

    def out_tail(layer, i):
        n = TO // NTO
        yns = [out_wo(layer, NSEG - 1, i * TO + u * n, n) for u in range(NTO)]
        for u in range(NTO):
            out_w1(NSEG - 1, i * TO + u * n, n, yns[u])

    def out_copy(t):
        rows = pl.ds(pl.multiple_of(t * TB, TB), TB)
        return pltpu.make_async_copy(obuf.at[rows], out_hbm.at[rows], sem_out.at[t])

    def b_step(t, layer):
        r = pl.multiple_of(t * TB, TB)
        hb = TB // NHALF
        x1s, x1ns = [], []
        for u in range(NHALF):
            ru = pl.multiple_of(r + u * hb, hb)
            parts = [hbuf[cb, pl.ds(ru + HPAD + SHIFTS[cb // 2], hb), :] for cb in range(D // 128)]
            x1 = ybuf[pl.ds(ru, hb), :] + _dot(jnp.concatenate(parts, axis=1).astype(BF16), w2[...])
            x1ns.append(_ln(x1))
            x1s.append(xmid[pl.ds(ru, hb), :] + x1)
        acc = jnp.concatenate(x1s, axis=0)
        x1n = jnp.concatenate(x1ns, axis=0).astype(BF16)
        for ci in range(F // FC):
            w3c = w3[:, ci * FC:(ci + 1) * FC]
            if ci == 0:
                h = jnp.concatenate([_gelu(_dot(part.astype(BF16), w3c)) for part in x1ns], axis=0).astype(BF16)
            else:
                h = _gelu(_dot(x1n, w3c)).astype(BF16)
            acc = acc + _dot(h, w4[ci * FC:(ci + 1) * FC, :])
        xres[pl.ds(r, TB), :] = acc
        obuf[pl.ds(r, TB), :] = acc.astype(BF16)

        @pl.when(layer == 1)
        def _():
            out_copy(t).start()

    def attn_phase(layer, p):
        @pl.when(jnp.logical_and(layer == 0, p == 0))
        def _():
            for g in (2, 3):
                group_wait(g)
            start_groups([4, 5, 6, 7])
            x_copy(2).start()

        @pl.when(jnp.logical_and(layer == 0, p == 1))
        def _():
            for g in (4, 5, 6, 7):
                group_wait(g)
            x_wait(2)
            cp_wo.start()
            cp_w1.start()
            x_copy(3).start()

        @pl.when(jnp.logical_and(layer == 0, p == 2))
        def _():
            cp_wo.wait()
            cp_w1.wait()
            x_wait(3)
            for cp in (cp_w2, cp_w3, cp_w4):
                cp.start()

        lo = jnp.where(p == 2, G, 2 * p)
        hi = jnp.where(p == 2, G + NPAIR + 2, jnp.where(p == 1, G, 2))
        loop(lo, hi, lambda j: attn_step(layer, j))

    def layer_body(layer):
        mt[...] = jnp.zeros(mt.shape, F32)
        zr[...] = jnp.zeros(zr.shape, F32)

        loop(0, 2, lambda b: layer_head(layer, b))
        loop(0, 3, lambda p: attn_phase(layer, p))
        loop(0, L // TO, lambda i: out_tail(layer, i))

        @pl.when(layer == 0)
        def _():
            cp_w2.wait()
            cp_w3.wait()
            cp_w4.wait()

        loop(0, NTB, lambda t: b_step(t, layer))

    loop(0, 2, layer_body)

    for t in range(NTB):
        out_copy(t).wait()


@jax.jit
def pallas_interleave_layers__memory_aug_infini_attn__mixer_s_mlp__prompt_kernel(
    A_x: jax.Array,
    A_wq: jax.Array,
    A_wk: jax.Array,
    A_wv: jax.Array,
    A_wo: jax.Array,
    A_beta: jax.Array,
    B_x: jax.Array,
    B_w1: jax.Array,
    B_w2: jax.Array,
    B_w3: jax.Array,
    B_w4: jax.Array,
):
    del B_x
    x = A_x.reshape(S, D)
    beta = A_beta.astype(F32)
    any_spec = pl.BlockSpec(memory_space=pl.ANY)
    scratch = [
        pltpu.VMEM((S, D), BF16),
        pltpu.VMEM((G, D, 128), BF16),
        pltpu.VMEM((G, D, 128), BF16),
        pltpu.VMEM((G, D, 128), BF16),
        pltpu.VMEM((D, D), BF16),
        pltpu.VMEM((D, D), BF16),
        pltpu.VMEM((D, D), BF16),
        pltpu.VMEM((D, F), BF16),
        pltpu.VMEM((F, D), BF16),
        pltpu.VMEM((G, 128, D), BF16),
        pltpu.VMEM((G, 128, D), BF16),
        pltpu.VMEM((S, D), F32),
        pltpu.VMEM((S, D), F32),
        pltpu.VMEM((S, D), BF16),
        pltpu.VMEM((S, D), F32),
        pltpu.VMEM((D // 128, S + 2 * HPAD, 128), F32),
        pltpu.VMEM((2, L, 128), BF16),
        pltpu.VMEM((2, L, 128), BF16),
        pltpu.VMEM((2, 128, L), BF16),
        pltpu.VMEM((2, 128, L), BF16),
        pltpu.VMEM((2, 128, L), BF16),
        pltpu.VMEM((2, G, L, 128), BF16),
        pltpu.VMEM((G, 128, 128), F32),
        pltpu.VMEM((G, 16, 128), F32),
        pltpu.VMEM((S, D), BF16),
        pltpu.VMEM((2, NQT * HPG, QT), F32),
        pltpu.VMEM((2 * RC, D), BF16),
        pltpu.VMEM((2 * RC, D), BF16),
        pltpu.SMEM((4,), F32),
        pltpu.SemaphoreType.DMA((NSEG,)),
        pltpu.SemaphoreType.DMA((G,)),
        pltpu.SemaphoreType.DMA((5,)),
        pltpu.SemaphoreType.DMA((NTB,)),
    ]
    out = pl.pallas_call(
        _kernel,
        out_shape=jax.ShapeDtypeStruct((S, D), BF16),
        in_specs=[pl.BlockSpec(memory_space=pltpu.SMEM)] + [any_spec] * 9,
        out_specs=any_spec,
        scratch_shapes=scratch,
        compiler_params=pltpu.CompilerParams(vmem_limit_bytes=120 * 1024 * 1024),
    )(beta, x, A_wq, A_wk, A_wv, A_wo, B_w1, B_w2, B_w3, B_w4)
    return out.reshape(1, S, D)
```

```python
import functools

import jax
import jax.numpy as jnp
from jax import lax
import jax.experimental.pallas as pl
import jax.experimental.pallas.tpu as pltpu

S = 2048
D = 1024
H = 32
DH = 32
NSEG = 4
L = 512
F = 3584
G = 8
HPG = 4
QT = 128
NQT = L // QT
HQ = QT // 2
HPAD = 8
FC = 512
RC = L // G
NP = 4
LN_AT = (1, 2, 3, 4)
STAGES = "x0 g0 x1 x6|g1 g2|g3 x2|g4 g5|g6 g7 x3|"
TB = 256
NTB = S // TB
NHALF = 2
X_PARTS = ((0, QT), (QT, QT), (L, L // 2), (3 * L // 2, L // 2), (2 * L, L), (3 * L, L), (L // 2, L // 2))
LOG2E = 1.4426950408889634
QSCALE = (DH ** -0.5) * LOG2E
MASK_BIAS = -1000000000.0 * LOG2E
GELU_C = 0.7978845608028654
SAFE_LOGIT = 40.0

F32 = jnp.float32
BF16 = jnp.bfloat16

NT = (((1,), (1,)), ((), ()))
SHIFTS = (-1, 1, -2, 2)
ORDER_FIRST = "cp S0 S1 P0 S2 P1 S3 P2 mr mu q P3 c k L02 v +S0 +S1 +P0 +S2 +P1 +S3 +P2 +mr +mu +q +P3 +c +k L12 +v"
ORDER_LAST = "S0 S1 P0 S2 P1 S3 P2 mr wo P3 c +S3 +S2 +P3 +S1 +P2 +S0 +mr +P1 +P0 +c w1"
ORDER_TAIL = "o01 o23 w01 w23"
ORDER_MID = "cp S0 S1 P0 S2 P1 S3 P2 mr mu q P3 c k L02 wo v +S0 +S1 +P0 +S2 +P1 +S3 +P2 +mr +mu +q +P3 +c +k L12 w1 +v"


def _ln(x):
    m = jnp.mean(x, axis=-1, keepdims=True)
    d = x - m
    v = jnp.mean(d * d, axis=-1, keepdims=True)
    return d * lax.rsqrt(v + 1e-05)


def _gelu(x):
    return 0.5 * x * (1.0 + jnp.tanh(GELU_C * (x + 0.044715 * (x * x * x))))


def _phi(t):
    return jnp.where(t > 0, t + 1.0, jnp.exp(t))


def _dot(a, b):
    return jnp.dot(a, b, preferred_element_type=F32)


def _kernel(beta_ref, x_hbm, wq_hbm, wk_hbm, wv_hbm, wo_hbm, w1_hbm, w2_hbm, w3_hbm, w4_hbm,
            out_hbm,
            xin, wq, wk, wv, wo, w1, w2, w3, w4, wqt, wvt,
            xres, xmid, xn, ybuf, hbuf, kb, pkb, qt, pqt, vt, ob, mt, zr, obuf, shift, lnb, amax,
            sem_x, sem_g, sem_w, sem_out):

    def x_copy(s):
        rows = pl.ds(*X_PARTS[s])
        return pltpu.make_async_copy(x_hbm.at[rows], xin.at[rows], sem_x.at[s])

    def group_copies(g):
        return [pltpu.make_async_copy(src.at[:, pl.ds(g * 128, 128)], dst.at[g], sem_g.at[g])
                for src, dst in ((wk_hbm, wk), (wq_hbm, wq), (wv_hbm, wv))]

    def group_wait(g):
        for cp in group_copies(g):
            cp.wait()

    w_pairs = [(wo_hbm, wo), (w1_hbm, w1), (w2_hbm, w2), (w3_hbm, w3), (w4_hbm, w4)]
    w_copies = [pltpu.make_async_copy(src, dst, sem_w.at[i]) for i, (src, dst) in enumerate(w_pairs)]
    cp_wo, cp_w1, cp_w2, cp_w3, cp_w4 = w_copies

    def stage(i):
        for item in STAGES.split("|")[i].split():
            for cp in [x_copy(int(item[1]))] if item[0] == "x" else group_copies(int(item[1])):
                cp.start()

    stage(0)

    hbuf[:, 0:HPAD, :] = jnp.zeros((D // 128, HPAD, 128), F32)
    hbuf[:, HPAD + S:HPAD + S + HPAD, :] = jnp.zeros((D // 128, HPAD, 128), F32)
    xres[0:TB, :] = jnp.zeros((TB, D), F32)

    def loop(lo, hi, fn):
        def body(i, c):
            fn(i)
            return c
        lax.fori_loop(lo, hi, body, 0)

    def aligned(i, n):
        return i if isinstance(i, int) else pl.multiple_of(i, n)

    def first_layer(layer, cond):
        return pl.when(cond) if layer == 0 else (lambda f: None)

    def residual(layer, rows):
        return xin[rows, :].astype(F32) if layer == 0 else xres[rows, :]

    def seg_rows(s):
        return pl.ds(s * L if isinstance(s, int) else pl.multiple_of(s * L, L), L)

    def proj_k(b, s, g):
        k = _dot(xn[seg_rows(s), :], wk[g])
        kb[b] = k.astype(BF16)
        pkb[b] = _phi(k).astype(BF16)
        amax[2 * b] = jnp.max(jnp.abs(k))

    def swap_halves(x):
        return jnp.concatenate([pltpu.roll(x[:, c:c + QT], HQ, 1) for c in range(0, x.shape[1], QT)], axis=1)

    def scaled_q(q):
        qs = q * QSCALE
        heads = [qs[h * DH:(h + 1) * DH, :] for h in range(HPG)]
        return jnp.concatenate([x if h % 2 else swap_halves(x) for h, x in enumerate(heads)], axis=0).astype(BF16)

    def proj_q(b, s, w):
        q = lax.dot_general(w, xn[seg_rows(s), :], NT, preferred_element_type=F32)
        qt[b] = scaled_q(q)
        pqt[b] = _phi(q).astype(BF16)
        amax[2 * b + 1] = jnp.max(jnp.abs(q))

    def proj_v(b, s, w):
        v = lax.dot_general(w, xn[seg_rows(s), :], NT, preferred_element_type=F32)
        vt[b] = v.astype(BF16)

    def transposed(src, dst, g):
        w = src[g].T
        dst[g] = w
        return w

    def store_proj(op, b, rows, y, mags):
        if op == "k":
            kb[b, rows, :] = y.astype(BF16)
            pkb[b, rows, :] = _phi(y).astype(BF16)
            mags[2 * b].append(jnp.max(jnp.abs(y), axis=0, keepdims=True))
        elif op == "q":
            mags[2 * b + 1].append(jnp.max(jnp.abs(y), axis=0, keepdims=True))
            q = y.T
            qt[b, :, rows] = scaled_q(q)
            pqt[b, :, rows] = _phi(q).astype(BF16)
        else:
            vt[b, :, rows] = y.T.astype(BF16)

    def first_head():
        weights = {"k": wk, "q": wq, "v": wv}
        mags = [[] for _ in range(2 * NP)]

        def fresh_rows(c, groups):
            rows = pl.ds(c * QT, QT)
            xc = _ln(residual(0, rows)).astype(BF16)
            xn[rows, :] = xc
            for b in groups:
                for op in "kqv":
                    store_proj(op, b, rows, _dot(xc, weights[op][b]), mags)

        def known_rows(n, b):
            for op in "qvk":
                store_proj(op, b, pl.ds(0, n), _dot(xn[0:n, :], weights[op][b]), mags)

        x_copy(0).wait()
        stage(1)
        xn[0:QT, :] = _ln(residual(0, pl.ds(0, QT))).astype(BF16)
        x_copy(1).wait()
        group_wait(0)
        stage(2)
        known_rows(QT, 0)
        fresh_rows(1, [0])
        x_copy(6).wait()
        stage(3)
        fresh_rows(2, [0])
        fresh_rows(3, [0])
        group_wait(1)
        stage(4)
        known_rows(L, 1)
        x_copy(2).wait()
        group_wait(2)
        group_wait(3)
        stage(5)
        lnb[...] = _ln(residual(0, pl.ds(L, NP * RC))).astype(BF16)
        known_rows(L, 2)
        known_rows(L, 3)
        for i, m in enumerate(mags):
            amax[i] = jnp.max(functools.reduce(jnp.maximum, m))

    def second_head():
        rows = pl.ds(S - TB, TB)
        xn[rows, :] = _ln(residual(1, rows)).astype(BF16)
        for b in range(NP):
            proj_q(b, 0, wqt[b])
            proj_k(b, 0, b)
            proj_v(b, 0, wvt[b])

    def out_wo(layer, s, r, n):
        rows = pl.ds(aligned(s * L + r, QT), n)
        rin = pl.ds(aligned(r, QT), n)
        o = jnp.concatenate([ob[s & 1, g, rin, :] for g in range(G)], axis=1)
        xm = residual(layer, rows) + _dot(o, wo[...])
        xmid[rows, :] = xm
        y = _ln(xm)
        ybuf[rows, :] = y
        return _ln(y).astype(BF16)

    def out_w1(s, r, n, yn):
        h = _gelu(_dot(yn, w1[...]))
        rows = pl.ds(aligned(HPAD + s * L + r, HPAD), n)
        for cb in range(D // 128):
            hbuf[cb, rows, :] = h[:, cb * 128:(cb + 1) * 128]

    def q_cols(b, queries):
        zero_blk = jnp.zeros((DH, QT), BF16)
        cols = []
        for h in range(HPG):
            blocks = [zero_blk] * HPG
            blocks[h] = qt[b, h * DH:(h + 1) * DH, queries]
            cols.append(jnp.concatenate(blocks, axis=0))
        return jnp.concatenate(cols, axis=1)

    def qk(b, i):
        return _dot(kb[b, 0:QT * i + HQ, :], q_cols(b, pl.ds(i * QT, QT)))

    def own_half(h, x, fill):
        lane = lax.broadcasted_iota(jnp.int32, x.shape, 1)
        return jnp.where(lane >= HQ if h % 2 else lane < HQ, x, fill)

    def qk_top(b, i):
        zero_half = jnp.zeros((DH, QT), jnp.uint32)
        blocks = [own_half(h, pltpu.bitcast(qt[b, h * DH:(h + 1) * DH, i * QT:(i + 1) * QT], jnp.uint32), 0)
                  for h in range(HPG)]
        pair = jnp.concatenate([jnp.concatenate(blocks[:2] + [zero_half], axis=0),
                                jnp.concatenate([zero_half] + blocks[2:], axis=0)], axis=1)
        return _dot(kb[b, QT * i + HQ:QT * (i + 1), :], pltpu.bitcast(pair, BF16))

    def causal_bias(nkeys, query):
        krow = lax.broadcasted_iota(jnp.int32, (nkeys, QT), 0)
        lane = lax.broadcasted_iota(jnp.int32, (nkeys, QT), 1)
        return jnp.where(krow > query(lane), MASK_BIAS, 0.0).astype(F32)

    def query_of(h):
        return (lambda lane: lane) if h % 2 else (lambda lane: (lane + HQ) & (QT - 1))

    def softmax_shift():
        scale = DH * QSCALE * 1.02
        safe = functools.reduce(jnp.logical_and,
                                [amax[2 * b] * amax[2 * b + 1] * scale <= SAFE_LOGIT for b in range(NP)])

        @pl.when(safe)
        def _():
            shift[...] = jnp.zeros(shift.shape, F32)

        @pl.when(jnp.logical_not(safe))
        def _():
            def row_max(t):
                b = lax.shift_right_logical(t, 2)
                i = t & (NQT - 1)
                q0 = pl.multiple_of(i * QT, QT)
                st = _dot(kb[b], q_cols(b, pl.ds(q0, QT)))
                for h in range(HPG):
                    sc = st[:, h * QT:(h + 1) * QT] + causal_bias(L, lambda lane: q0 + query_of(h)(lane))
                    shift[b, pl.ds(i * HPG + h, 1), :] = jnp.max(sc, axis=0, keepdims=True)
            loop(0, NP * NQT, row_max)

    def probs(b, i):
        lo = qk(b, i)
        hi = qk_top(b, i)
        nd = QT * i
        shifts = [shift[b, i * HPG + h:i * HPG + h + 1, :] for h in range(HPG)]
        res = []
        for h in range(HPG):
            if h % 2 == 0:
                top = hi[:, (h // 2) * QT:(h // 2 + 1) * QT] + causal_bias(HQ, lambda lane: lane & (HQ - 1))
                top = jnp.exp2(top - own_half(h, shifts[h], shifts[h + 1]))
                top_sum = jnp.sum(top, axis=0, keepdims=True)
            sc = lo[:, h * QT:(h + 1) * QT]
            diag = sc[nd:, :] + causal_bias(HQ, query_of(h))
            p = jnp.exp2((diag if i == 0 else jnp.concatenate([sc[:nd, :], diag], axis=0)) - shifts[h])
            total = jnp.sum(p, axis=0, keepdims=True) + own_half(h, top_sum, 0.0)
            res.append((jnp.concatenate([p, own_half(h, top, 0.0)], axis=0).astype(BF16), total))
        return res

    def pv(b, i, ps):
        nk = QT * (i + 1)
        return [(_dot(vt[b, h * DH:(h + 1) * DH, 0:nk], ps[h][0]), ps[h][1]) for h in range(HPG)]

    def mem_read(b, g):
        mem = jnp.concatenate([mt[g], zr[g]], axis=0).astype(BF16)
        return _dot(mem, pqt[b])

    def mem_update(b, g):
        vaug = jnp.concatenate([vt[b], jnp.ones((16, L), BF16)], axis=0)
        upd = _dot(vaug, pkb[b])
        rh = lax.broadcasted_iota(jnp.int32, (144, 128), 0)
        ch = lax.broadcasted_iota(jnp.int32, (144, 128), 1) // DH
        upd = jnp.where(jnp.where(rh < 128, rh // DH, rh - 128) == ch, upd, 0.0)
        mt[g] = mt[g] + upd[:128]
        zr[g] = zr[g] + upd[128:]

    def combine(s, g, nd, res):
        rows = []
        for h in range(HPG):
            gate = jax.nn.sigmoid(jnp.full((1, L), beta_ref[g * HPG + h], F32))
            l_h = jnp.concatenate([res[i][h][1] for i in range(NQT)], axis=1)
            o_h = jnp.concatenate([res[i][h][0] for i in range(NQT)], axis=1)
            c_dot = (1.0 - gate) / l_h
            c_mem = gate / (nd[128 + h:129 + h, :] + 1e-06)
            o_h = c_dot * o_h
            rows.append(c_mem * nd[h * DH:(h + 1) * DH, :] + (o_h if h % 2 else swap_halves(o_h)))
        ob[s & 1, g] = jnp.concatenate(rows, axis=0).T.astype(BF16)

    def run(layer, order, j, fresh):
        n = 2 * RC
        s = j >> 3
        last_rows = S - NP * RC
        state = [({}, {}, {}) for _ in range(NP)]
        shared = {}
        ops = [(op.lstrip("+"), base + op.count("+")) for base in range(0, NP, 2) for op in order.split()]
        for op, b in ops:
            ps, res, tmp = state[b]
            g = (j + b) & (G - 1)
            sn = (j + b + NP) >> 3
            gn = (j + b + NP) & (G - 1)
            if op[0] == "S":
                ps[int(op[1])] = probs(b, int(op[1]))
            elif op[0] == "P":
                res[int(op[1])] = pv(b, int(op[1]), ps[int(op[1])])
            elif op == "mr":
                tmp["nd"] = mem_read(b, g)
            elif op == "mu":
                mem_update(b, g)
            elif op == "wo":
                shared["yn"] = out_wo(layer, s - 1, g * RC, n)
            elif op == "w1":
                out_w1(s - 1, g * RC, n, shared["yn"])
            elif op == "q":
                proj_q(b, sn, transposed(wq, wqt, gn) if fresh else wqt[gn])
            elif op == "k":
                proj_k(b, sn, gn)
            elif op == "v":
                proj_v(b, sn, transposed(wv, wvt, gn) if fresh else wvt[gn])
            elif op[0] == "L" and layer == 0:
                m = n // int(op[2])
                off = b * RC + int(op[1]) * m
                rows = pl.ds(pl.multiple_of(jnp.minimum((j + G + NP) * RC, last_rows) + off, m), m)
                lnb[off:off + m, :] = _ln(residual(layer, rows)).astype(BF16)
            elif op == "cp" and layer == 0 and b == 0:
                rows = pl.ds(pl.multiple_of(jnp.minimum((j + G) * RC, last_rows), NP * RC), NP * RC)
                xn[rows, :] = lnb[...]
            elif op == "c":
                combine(s, g, tmp["nd"], res)

    def attn_step(layer, order, it, fresh=False):
        softmax_shift()
        run(layer, order, it * NP if isinstance(it, int) else pl.multiple_of(it * NP, NP), fresh)

    def first_step(layer, it):
        @first_layer(layer, it == 0)
        def _():
            for g in range(NP, G):
                group_wait(g)
            x_copy(3).wait()
            x_copy(4).start()

        @first_layer(layer, it == 1)
        def _():
            x_copy(4).wait()
            cp_wo.start()
            cp_w1.start()
            x_copy(5).start()

        attn_step(layer, ORDER_FIRST, it, layer == 0)

    def last_step(layer):
        attn_step(layer, ORDER_LAST, NSEG * G // NP - 1)
        yns = {}
        for op in ORDER_TAIL.split():
            r, n = int(op[1]) * QT, (int(op[-1]) - int(op[1]) + 1) * QT
            if op[0] == "o":
                yns[op[1:]] = out_wo(layer, NSEG - 1, r, n)
            else:
                out_w1(NSEG - 1, r, n, yns[op[1:]])

    def out_copy(t):
        rows = pl.ds(pl.multiple_of(t * TB, TB), TB)
        return pltpu.make_async_copy(obuf.at[rows], out_hbm.at[rows], sem_out.at[t])

    def b_step(t, layer):
        r = pl.multiple_of(t * TB, TB)
        hb = TB // NHALF
        x1s, x1ns = [], []
        for u in range(NHALF):
            ru = pl.multiple_of(r + u * hb, hb)
            parts = [hbuf[cb, pl.ds(ru + HPAD + SHIFTS[cb // 2], hb), :] for cb in range(D // 128)]
            x1 = ybuf[pl.ds(ru, hb), :] + _dot(jnp.concatenate(parts, axis=1).astype(BF16), w2[...])
            x1ns.append(_ln(x1))
            x1s.append(xmid[pl.ds(ru, hb), :] + x1)
        acc = jnp.concatenate(x1s, axis=0)
        x1n = jnp.concatenate(x1ns, axis=0).astype(BF16)
        for ci in range(F // FC):
            if layer == 0 and ci in LN_AT:
                m = TB // len(LN_AT)
                off = LN_AT.index(ci) * m
                prev = pl.ds(pl.multiple_of(jnp.maximum(r - TB, 0) + off, m), m)
                normed = _ln(xres[prev, :])
                xn[prev, :] = normed.astype(BF16)
                pieces = [acc[:off], jnp.where(t < 0, normed, acc[off:off + m]), acc[off + m:]]
                acc = jnp.concatenate([p for p in pieces if p.shape[0]], axis=0)
            w3c = w3[:, ci * FC:(ci + 1) * FC]
            if ci == 0:
                h = jnp.concatenate([_gelu(_dot(part.astype(BF16), w3c)) for part in x1ns], axis=0).astype(BF16)
            else:
                h = _gelu(_dot(x1n, w3c)).astype(BF16)
            acc = acc + _dot(h, w4[ci * FC:(ci + 1) * FC, :])
        if layer == 0:
            xres[pl.ds(r, TB), :] = acc
        else:
            obuf[pl.ds(r, TB), :] = acc.astype(BF16)
            out_copy(t).start()

    def layer_body(layer):
        mt[...] = jnp.zeros(mt.shape, F32)
        zr[...] = jnp.zeros(zr.shape, F32)

        (first_head if layer == 0 else second_head)()
        loop(0, G // NP, lambda it: first_step(layer, it))
        if layer == 0:
            cp_wo.wait()
            cp_w1.wait()
            x_copy(5).wait()
            for cp in (cp_w2, cp_w3, cp_w4):
                cp.start()
        loop(G // NP, NSEG * G // NP - 1, lambda it: attn_step(layer, ORDER_MID, it))
        last_step(layer)

        if layer == 0:
            cp_w2.wait()
            cp_w3.wait()
            cp_w4.wait()

        loop(0, NTB, lambda t: b_step(t, layer))

    for layer in range(2):
        layer_body(layer)

    for t in range(NTB):
        out_copy(t).wait()


@jax.jit
def pallas_interleave_layers__memory_aug_infini_attn__mixer_s_mlp__prompt_kernel(
    A_x: jax.Array,
    A_wq: jax.Array,
    A_wk: jax.Array,
    A_wv: jax.Array,
    A_wo: jax.Array,
    A_beta: jax.Array,
    B_x: jax.Array,
    B_w1: jax.Array,
    B_w2: jax.Array,
    B_w3: jax.Array,
    B_w4: jax.Array,
):
    del B_x
    x = A_x.reshape(S, D)
    beta = A_beta.astype(F32)
    any_spec = pl.BlockSpec(memory_space=pl.ANY)
    scratch = [
        pltpu.VMEM((S, D), BF16),
        pltpu.VMEM((G, D, 128), BF16),
        pltpu.VMEM((G, D, 128), BF16),
        pltpu.VMEM((G, D, 128), BF16),
        pltpu.VMEM((D, D), BF16),
        pltpu.VMEM((D, D), BF16),
        pltpu.VMEM((D, D), BF16),
        pltpu.VMEM((D, F), BF16),
        pltpu.VMEM((F, D), BF16),
        pltpu.VMEM((G, 128, D), BF16),
        pltpu.VMEM((G, 128, D), BF16),
        pltpu.VMEM((S, D), F32),
        pltpu.VMEM((S, D), F32),
        pltpu.VMEM((S, D), BF16),
        pltpu.VMEM((S, D), F32),
        pltpu.VMEM((D // 128, S + 2 * HPAD, 128), F32),
        pltpu.VMEM((NP, L, 128), BF16),
        pltpu.VMEM((NP, L, 128), BF16),
        pltpu.VMEM((NP, 128, L), BF16),
        pltpu.VMEM((NP, 128, L), BF16),
        pltpu.VMEM((NP, 128, L), BF16),
        pltpu.VMEM((2, G, L, 128), BF16),
        pltpu.VMEM((G, 128, 128), F32),
        pltpu.VMEM((G, 16, 128), F32),
        pltpu.VMEM((S, D), BF16),
        pltpu.VMEM((NP, NQT * HPG, QT), F32),
        pltpu.VMEM((NP * RC, D), BF16),
        pltpu.SMEM((2 * NP,), F32),
        pltpu.SemaphoreType.DMA((len(X_PARTS),)),
        pltpu.SemaphoreType.DMA((G,)),
        pltpu.SemaphoreType.DMA((5,)),
        pltpu.SemaphoreType.DMA((NTB,)),
    ]
    out = pl.pallas_call(
        _kernel,
        out_shape=jax.ShapeDtypeStruct((S, D), BF16),
        in_specs=[pl.BlockSpec(memory_space=pltpu.SMEM)] + [any_spec] * 9,
        out_specs=any_spec,
        scratch_shapes=scratch,
        compiler_params=pltpu.CompilerParams(vmem_limit_bytes=120 * 1024 * 1024),
    )(beta, x, A_wq, A_wk, A_wv, A_wo, B_w1, B_w2, B_w3, B_w4)
    return out.reshape(1, S, D)
```

```python
import functools

import jax
import jax.numpy as jnp
from jax import lax
import jax.experimental.pallas as pl
import jax.experimental.pallas.tpu as pltpu

S = 2048
D = 1024
H = 32
DH = 32
NSEG = 4
L = 512
F = 3584
G = 8
HPG = 4
QT = 128
NQT = L // QT
HQ = QT // 2
HPAD = 8
FC = 512
RC = L // G
NP = 4
LN_AT = (1, 2, 3, 4)
STAGES = "x0 g0 x1 x6|g1 g2|g3 g4|g5 x2|g6 g7 x3|"
TB = 256
NTB = S // TB
HEAD_T = "123"
FIRST_LN = [RC * int(c) for c in "00212111"]
LOOP_LN = [RC * int(c) for c in "01010101"]
OUT_R = 128
OUT_C = 512
OUT_PIECES = [(r, c) for r in range(0, TB, OUT_R) for c in range(0, D, OUT_C)]
NOUT = len(OUT_PIECES)
NHALF = 2
X_PARTS = ((0, QT), (QT, QT), (L, L // 2), (3 * L // 2, L // 2), (2 * L, L // 2), (5 * L // 2, 3 * L // 2), (L // 2, L // 2))
LOG2E = 1.4426950408889634
QSCALE = (DH ** -0.5) * LOG2E
MASK_BIAS = -1000000000.0 * LOG2E
GELU_C = 0.7978845608028654
SAFE_LOGIT = 40.0

F32 = jnp.float32
BF16 = jnp.bfloat16

NT = (((1,), (1,)), ((), ()))
SHIFTS = (-1, 1, -2, 2)
ORDER_FIRST = "S0 S1 P0 S2 P1 S3 P2 mr mu q L P3 c k L v W +S0 +S1 +P0 +S2 +P1 +S3 +P2 +mr +mu +q L +P3 +c +k L +v"
ORDER_LAST = "S0 S1 P0 S2 P1 S3 P2 mr wo P3 c +S3 +S2 +P3 +S1 +P2 +S0 +mr +P1 +P0 +c w1"
ORDER_TAIL = "o01 o23 m0 w01 w23"
ORDER_MID = "cp S0 S1 P0 S2 P1 S3 P2 mr mu q L P3 c k L wo v +S0 +S1 +P0 +S2 +P1 +S3 +P2 +mr +mu +q L +P3 +c +k L w1 +v"


def _ln(x):
    m = jnp.mean(x, axis=-1, keepdims=True)
    d = x - m
    v = jnp.mean(d * d, axis=-1, keepdims=True)
    return d * lax.rsqrt(v + 1e-05)


def _gelu(x):
    return 0.5 * x * (1.0 + jnp.tanh(GELU_C * (x + 0.044715 * (x * x * x))))


def _phi(t):
    return jnp.where(t > 0, t + 1.0, jnp.exp(t))


def _dot(a, b):
    return jnp.dot(a, b, preferred_element_type=F32)


def _kernel(beta_hbm, x_hbm, wq_hbm, wk_hbm, wv_hbm, wo_hbm, w1_hbm, w2_hbm, w3_hbm, w4_hbm,
            out_hbm,
            xin, wq, wk, wv, wo, w1, w2, w3, w4, wqt, wvt,
            xres, xmid, xn, ybuf, hbuf, kb, pkb, qt, pqt, vt, ob, mt, zr, obuf, shift, lnb, x1b, beta_in, beta, amax,
            sem_x, sem_g, sem_w, sem_out):

    def x_copy(s):
        rows = pl.ds(*X_PARTS[s])
        return pltpu.make_async_copy(x_hbm.at[rows], xin.at[rows], sem_x.at[s])

    def group_copies(g):
        return [pltpu.make_async_copy(src.at[:, pl.ds(g * 128, 128)], dst.at[g], sem_g.at[g])
                for src, dst in ((wk_hbm, wk), (wq_hbm, wq), (wv_hbm, wv))]

    def group_wait(g):
        for cp in group_copies(g):
            cp.wait()

    w_pairs = [(wo_hbm, wo), (w1_hbm, w1), (w2_hbm, w2), (w3_hbm, w3), (w4_hbm, w4), (beta_hbm, beta_in)]
    w_copies = [pltpu.make_async_copy(src, dst, sem_w.at[i]) for i, (src, dst) in enumerate(w_pairs)]
    cp_wo, cp_w1, cp_w2, cp_w3, cp_w4, cp_beta = w_copies

    def stage(i):
        for item in STAGES.split("|")[i].split():
            for cp in [x_copy(int(item[1]))] if item[0] == "x" else group_copies(int(item[1])):
                cp.start()

    cp_beta.start()
    stage(0)

    hbuf[:, 0:HPAD, :] = jnp.zeros((D // 128, HPAD, 128), F32)
    hbuf[:, HPAD + S:HPAD + S + HPAD, :] = jnp.zeros((D // 128, HPAD, 128), F32)
    xres[0:TB, :] = jnp.zeros((TB, D), F32)
    shift[...] = jnp.zeros(shift.shape, F32)
    amax[2 * NP] = 0.0

    def loop(lo, hi, fn):
        def body(i, c):
            fn(i)
            return c
        lax.fori_loop(lo, hi, body, 0)

    def aligned(i, n):
        return i if isinstance(i, int) else pl.multiple_of(i, n)

    def residual(layer, rows):
        return xin[rows, :].astype(F32) if layer == 0 else xres[rows, :]

    def seg_rows(s):
        return pl.ds(s * L if isinstance(s, int) else pl.multiple_of(s * L, L), L)

    def proj_k(b, s, g):
        k = _dot(xn[seg_rows(s), :], wk[g])
        kb[b] = k.astype(BF16)
        pkb[b] = _phi(k).astype(BF16)
        amax[2 * b] = mag = jnp.max(jnp.abs(k))
        return mag

    def swap_halves(x):
        return jnp.concatenate([pltpu.roll(x[:, c:c + QT], HQ, 1) for c in range(0, x.shape[1], QT)], axis=1)

    def scaled_q(q):
        qs = q * QSCALE
        heads = [qs[h * DH:(h + 1) * DH, :] for h in range(HPG)]
        return jnp.concatenate([x if h % 2 else swap_halves(x) for h, x in enumerate(heads)], axis=0).astype(BF16)

    def proj_q(b, s, w):
        q = lax.dot_general(w, xn[seg_rows(s), :], NT, preferred_element_type=F32)
        qt[b] = scaled_q(q)
        pqt[b] = _phi(q).astype(BF16)
        amax[2 * b + 1] = mag = jnp.max(jnp.abs(q))
        return mag

    def proj_v(b, s, w):
        v = lax.dot_general(w, xn[seg_rows(s), :], NT, preferred_element_type=F32)
        vt[b] = v.astype(BF16)

    def zero_after(mag):
        return 0 if mag is None else (mag < 0.0).astype(jnp.int32)

    def transposed(src, dst, g, mag=None):
        w = src[g ^ zero_after(mag)].T
        dst[g] = w
        return w

    def store_proj(op, b, rows, y, mags):
        if op == "k":
            kb[b, rows, :] = y.astype(BF16)
            pkb[b, rows, :] = _phi(y).astype(BF16)
            mags[2 * b].append(jnp.max(jnp.abs(y), axis=0, keepdims=True))
        elif op == "q":
            mags[2 * b + 1].append(jnp.max(jnp.abs(y), axis=0, keepdims=True))
            q = y.T
            qt[b, :, rows] = scaled_q(q)
            pqt[b, :, rows] = _phi(q).astype(BF16)
        else:
            vt[b, :, rows] = y.T.astype(BF16)

    def first_head():
        weights = {"k": wk, "q": wq, "v": wv}
        mags = [[] for _ in range(2 * NP)]

        def fresh_rows(c, groups):
            rows = pl.ds(c * QT, QT)
            xc = _ln(residual(0, rows)).astype(BF16)
            xn[rows, :] = xc
            for b in groups:
                for op in "kqv":
                    store_proj(op, b, rows, _dot(xc, weights[op][b]), mags)

        def known_rows(n, b):
            if str(b) in HEAD_T:
                proj_k(b, 0, b)
                proj_q(b, 0, transposed(wq, wqt, b))
                proj_v(b, 0, transposed(wv, wvt, b))
                return
            for op in "qvk":
                store_proj(op, b, pl.ds(0, n), _dot(xn[0:n, :], weights[op][b]), mags)

        cp_beta.wait()
        head_of = lax.broadcasted_iota(jnp.int32, (1, H), 1)
        betas = beta_in[...].astype(F32).reshape(1, H)
        for h in range(H):
            beta[h] = jnp.sum(jnp.where(head_of == h, betas, 0.0))
        x_copy(0).wait()
        stage(1)
        xn[0:QT, :] = _ln(residual(0, pl.ds(0, QT))).astype(BF16)
        x_copy(1).wait()
        group_wait(0)
        stage(2)
        known_rows(QT, 0)
        fresh_rows(1, [0])
        x_copy(6).wait()
        stage(3)
        fresh_rows(2, [0])
        fresh_rows(3, [0])
        group_wait(1)
        stage(4)
        known_rows(L, 1)
        group_wait(2)
        group_wait(3)
        stage(5)
        known_rows(L, 2)
        known_rows(L, 3)
        for i, m in enumerate(mags):
            if m:
                amax[i] = jnp.max(functools.reduce(jnp.maximum, m))

    def second_head():
        rows = pl.ds(S - TB, TB)
        xn[rows, :] = _ln(residual(1, rows)).astype(BF16)
        for b in range(NP):
            proj_q(b, 0, wqt[b])
            proj_k(b, 0, b)
            proj_v(b, 0, wvt[b])

    def out_wo(layer, s, r, n):
        rows = pl.ds(aligned(s * L + r, QT), n)
        rin = pl.ds(aligned(r, QT), n)
        o = jnp.concatenate([ob[s & 1, g, rin, :] for g in range(G)], axis=1)
        xm = residual(layer, rows) + _dot(o, wo[...])
        xmid[rows, :] = xm
        y = _ln(xm)
        ybuf[rows, :] = y
        return _ln(y).astype(BF16)

    def out_w1(s, r, n, yn):
        h = _gelu(_dot(yn, w1[...]))
        rows = pl.ds(aligned(HPAD + s * L + r, HPAD), n)
        for cb in range(D // 128):
            hbuf[cb, rows, :] = h[:, cb * 128:(cb + 1) * 128]

    def q_cols(b, queries):
        zero_blk = jnp.zeros((DH, QT), BF16)
        cols = []
        for h in range(HPG):
            blocks = [zero_blk] * HPG
            blocks[h] = qt[b, h * DH:(h + 1) * DH, queries]
            cols.append(jnp.concatenate(blocks, axis=0))
        return jnp.concatenate(cols, axis=1)

    def qk(b, i):
        return _dot(kb[b, 0:QT * i + HQ, :], q_cols(b, pl.ds(i * QT, QT)))

    def own_half(h, x, fill):
        lane = lax.broadcasted_iota(jnp.int32, x.shape, 1)
        return jnp.where(lane >= HQ if h % 2 else lane < HQ, x, fill)

    def qk_top(b, i):
        zero_half = jnp.zeros((DH, QT), jnp.uint32)
        blocks = [own_half(h, pltpu.bitcast(qt[b, h * DH:(h + 1) * DH, i * QT:(i + 1) * QT], jnp.uint32), 0)
                  for h in range(HPG)]
        pair = jnp.concatenate([jnp.concatenate(blocks[:2] + [zero_half], axis=0),
                                jnp.concatenate([zero_half] + blocks[2:], axis=0)], axis=1)
        return _dot(kb[b, QT * i + HQ:QT * (i + 1), :], pltpu.bitcast(pair, BF16))

    def causal_bias(nkeys, query):
        krow = lax.broadcasted_iota(jnp.int32, (nkeys, QT), 0)
        lane = lax.broadcasted_iota(jnp.int32, (nkeys, QT), 1)
        return jnp.where(krow > query(lane), MASK_BIAS, 0.0).astype(F32)

    def query_of(h):
        return (lambda lane: lane) if h % 2 else (lambda lane: (lane + HQ) & (QT - 1))

    def softmax_shift():
        scale = DH * QSCALE * 1.02
        safe = functools.reduce(jnp.logical_and,
                                [amax[2 * b] * amax[2 * b + 1] * scale <= SAFE_LOGIT for b in range(NP)],
                                amax[2 * NP] == 0.0)

        @pl.when(jnp.logical_not(safe))
        def _():
            amax[2 * NP] = 1.0

            def row_max(t):
                b = lax.shift_right_logical(t, 2)
                i = t & (NQT - 1)
                q0 = pl.multiple_of(i * QT, QT)
                st = _dot(kb[b], q_cols(b, pl.ds(q0, QT)))
                for h in range(HPG):
                    sc = st[:, h * QT:(h + 1) * QT] + causal_bias(L, lambda lane: q0 + query_of(h)(lane))
                    shift[b, pl.ds(i * HPG + h, 1), :] = jnp.max(sc, axis=0, keepdims=True)
            loop(0, NP * NQT, row_max)

    def probs(b, i):
        lo = qk(b, i)
        hi = qk_top(b, i)
        nd = QT * i
        shifts = [shift[b, i * HPG + h:i * HPG + h + 1, :] for h in range(HPG)]
        res = []
        for h in range(HPG):
            if h % 2 == 0:
                top = hi[:, (h // 2) * QT:(h // 2 + 1) * QT] + causal_bias(HQ, lambda lane: lane & (HQ - 1))
                top = jnp.exp2(top - own_half(h, shifts[h], shifts[h + 1]))
                top_sum = jnp.sum(top, axis=0, keepdims=True)
            sc = lo[:, h * QT:(h + 1) * QT]
            diag = sc[nd:, :] + causal_bias(HQ, query_of(h))
            p = jnp.exp2((diag if i == 0 else jnp.concatenate([sc[:nd, :], diag], axis=0)) - shifts[h])
            total = jnp.sum(p, axis=0, keepdims=True) + own_half(h, top_sum, 0.0)
            res.append((jnp.concatenate([p, own_half(h, top, 0.0)], axis=0).astype(BF16), total))
        return res

    def pv(b, i, ps):
        nk = QT * (i + 1)
        return [(_dot(vt[b, h * DH:(h + 1) * DH, 0:nk], ps[h][0]), ps[h][1]) for h in range(HPG)]

    def mem_read(b, g):
        mem = jnp.concatenate([mt[g], zr[g]], axis=0).astype(BF16)
        return _dot(mem, pqt[b])

    def mem_update(b, g):
        vaug = jnp.concatenate([vt[b], jnp.ones((16, L), BF16)], axis=0)
        upd = _dot(vaug, pkb[b])
        rh = lax.broadcasted_iota(jnp.int32, (144, 128), 0)
        ch = lax.broadcasted_iota(jnp.int32, (144, 128), 1) // DH
        upd = jnp.where(jnp.where(rh < 128, rh // DH, rh - 128) == ch, upd, 0.0)
        mt[g] = mt[g] + upd[:128]
        zr[g] = zr[g] + upd[128:]

    def combine(s, g, nd, res):
        rows = []
        for h in range(HPG):
            gate = jax.nn.sigmoid(jnp.full((1, L), beta[g * HPG + h], F32))
            l_h = jnp.concatenate([res[i][h][1] for i in range(NQT)], axis=1)
            o_h = jnp.concatenate([res[i][h][0] for i in range(NQT)], axis=1)
            c_dot = (1.0 - gate) / l_h
            c_mem = gate / (nd[128 + h:129 + h, :] + 1e-06)
            o_h = c_dot * o_h
            rows.append(c_mem * nd[h * DH:(h + 1) * DH, :] + (o_h if h % 2 else swap_halves(o_h)))
        ob[s & 1, g] = jnp.concatenate(rows, axis=0).T.astype(BF16)

    def run(layer, order, j, fresh):
        n = 2 * RC
        s = j >> 3
        last_rows = S - NP * RC
        state = [({}, {}, {}) for _ in range(NP)]
        shared = {}
        ops = [(op.lstrip("+"), base + op.count("+")) for base in range(0, NP, 2) for op in order.split()]
        for op, b in ops:
            ps, res, tmp = state[b]
            g = (j + b) & (G - 1)
            sn = (j + b + NP) >> 3
            gn = (j + b + NP) & (G - 1)
            if op[0] == "S":
                ps[int(op[1])] = probs(b, int(op[1]))
            elif op[0] == "P":
                res[int(op[1])] = pv(b, int(op[1]), ps[int(op[1])])
            elif op == "mr":
                tmp["nd"] = mem_read(b, g)
            elif op == "mu":
                mem_update(b, g)
            elif op == "wo":
                shared["yn"] = out_wo(layer, s - 1, g * RC, n)
            elif op == "w1":
                out_w1(s - 1, g * RC, n, shared["yn"])
            elif op == "q":
                shared["q"] = shared["mag"] = proj_q(b, sn, transposed(wq, wqt, gn, shared.get("q")) if fresh and str(gn) not in HEAD_T else wqt[gn])
            elif op == "k":
                shared["mag"] = proj_k(b, sn, gn)
            elif op == "v":
                proj_v(b, sn, transposed(wv, wvt, gn, shared["q"]) if fresh and str(gn) not in HEAD_T else wvt[gn])
            elif op == "L" and layer == 0:
                sizes = FIRST_LN if fresh and j == 0 else LOOP_LN
                idx = shared["ln"] = shared.get("ln", -1) + 1
                m, off = sizes[idx], sum(sizes[:idx])
                if m:
                    start = L if fresh and j == 0 else jnp.minimum((j + G + NP) * RC, last_rows)
                    after = zero_after(shared["mag"]) * RC if fresh else 0
                    y = _ln(residual(layer, pl.ds(pl.multiple_of(start + off - after, RC), m))).astype(BF16)
                    if fresh and j == 0:
                        xn[L + off:L + off + m, :] = y
                    else:
                        lnb[off:off + m, :] = y
            elif op == "cp" and layer == 0 and b == 0 and not fresh:
                rows = pl.ds(pl.multiple_of(jnp.minimum((j + G) * RC, last_rows), NP * RC), NP * RC)
                xn[rows, :] = lnb[...]
            elif op == "W" and layer == 0 and b == 0 and j == 0:
                for cp in [x_copy(2), x_copy(3)] + group_copies(6) + group_copies(7):
                    cp.wait()
            elif op == "c":
                combine(s, g, tmp["nd"], res)

    def attn_step(layer, order, it, fresh=False):
        softmax_shift()
        run(layer, order, it * NP if isinstance(it, int) else pl.multiple_of(it * NP, NP), fresh)

    def first_steps():
        group_wait(4)
        group_wait(5)
        x_copy(4).start()
        attn_step(0, ORDER_FIRST, 0, True)
        x_copy(4).wait()
        cp_wo.start()
        cp_w1.start()
        x_copy(5).start()
        attn_step(0, ORDER_FIRST, 1, True)

    def last_step(layer):
        attn_step(layer, ORDER_LAST, NSEG * G // NP - 1)
        yns = {}
        for op in ORDER_TAIL.split():
            r, n = int(op[1]) * QT, (int(op[-1]) - int(op[1]) + 1) * QT
            if op[0] == "m":
                mix(0)
            elif op[0] == "o":
                yns[op[1:]] = out_wo(layer, NSEG - 1, r, n)
            else:
                out_w1(NSEG - 1, r, n, yns[op[1:]])

    def out_copy(t):
        rows = pl.ds(aligned(t * TB, TB), TB)
        return pltpu.make_async_copy(obuf.at[rows], out_hbm.at[rows], sem_out.at[t])

    def out_piece(c):
        part = (pl.ds(S - TB + OUT_PIECES[c][0], OUT_R), pl.ds(OUT_PIECES[c][1], OUT_C))
        return pltpu.make_async_copy(obuf.at[part], out_hbm.at[part], sem_out.at[NTB - 1 + c])

    def mix(t):
        hb = TB // NHALF
        for u in range(NHALF):
            ru = aligned(t * TB + u * hb, hb)
            parts = [hbuf[cb, pl.ds(ru + HPAD + SHIFTS[cb // 2], hb), :] for cb in range(D // 128)]
            x1 = ybuf[pl.ds(ru, hb), :] + _dot(jnp.concatenate(parts, axis=1).astype(BF16), w2[...])
            x1b[u * hb:(u + 1) * hb, :] = _ln(x1).astype(BF16)
            xmid[pl.ds(ru, hb), :] = xmid[pl.ds(ru, hb), :] + x1

    def b_step(t, layer, ahead):
        r = aligned(t * TB, TB)
        acc = xmid[pl.ds(r, TB), :]
        for ci in range(F // FC):
            if layer == 0 and ci in LN_AT:
                m = TB // len(LN_AT)
                off = LN_AT.index(ci) * m
                prev = pl.ds(pl.multiple_of(jnp.maximum(r - TB, 0) + off, m), m)
                normed = _ln(xres[prev, :])
                xn[prev, :] = normed.astype(BF16)
                pieces = [acc[:off], jnp.where(amax[0] < 0, normed, acc[off:off + m]), acc[off + m:]]
                acc = jnp.concatenate([p for p in pieces if p.shape[0]], axis=0)
            h = _gelu(_dot(x1b[...], w3[:, ci * FC:(ci + 1) * FC])).astype(BF16)
            if ahead and ci == F // FC - 1:
                mix(t + 1)
            if layer == 1 and not ahead and ci == F // FC - 1:
                for c, (r0, c0) in enumerate(OUT_PIECES):
                    rows, cols = slice(r0, r0 + OUT_R), slice(c0, c0 + OUT_C)
                    piece = acc[rows, cols] + _dot(h[rows], w4[ci * FC:(ci + 1) * FC, cols])
                    obuf[pl.ds(r + r0, OUT_R), cols] = piece.astype(BF16)
                    out_piece(c).start()
                return
            acc = acc + _dot(h, w4[ci * FC:(ci + 1) * FC, :])
        if layer == 0:
            xres[pl.ds(r, TB), :] = acc
        else:
            obuf[pl.ds(r, TB), :] = acc.astype(BF16)
            out_copy(t).start()

    def layer_body(layer):
        mt[...] = jnp.zeros(mt.shape, F32)
        zr[...] = jnp.zeros(zr.shape, F32)

        (first_head if layer == 0 else second_head)()
        if layer == 1:
            loop(0, G // NP, lambda it: attn_step(layer, ORDER_FIRST, it))
        else:
            first_steps()
            cp_wo.wait()
            cp_w1.wait()
            x_copy(5).wait()
            for cp in (cp_w2, cp_w3, cp_w4):
                cp.start()
        loop(G // NP, NSEG * G // NP - 1, lambda it: attn_step(layer, ORDER_MID, it))
        if layer == 0:
            cp_w2.wait()
            cp_w3.wait()
            cp_w4.wait()
        last_step(layer)
        loop(0, NTB - 1, lambda t: b_step(t, layer, True))
        b_step(NTB - 1, layer, False)

    for layer in range(2):
        layer_body(layer)

    for t in range(NTB - 1):
        out_copy(t).wait()
    for c in range(NOUT):
        out_piece(c).wait()


@jax.jit
def pallas_interleave_layers__memory_aug_infini_attn__mixer_s_mlp__prompt_kernel(
    A_x: jax.Array,
    A_wq: jax.Array,
    A_wk: jax.Array,
    A_wv: jax.Array,
    A_wo: jax.Array,
    A_beta: jax.Array,
    B_x: jax.Array,
    B_w1: jax.Array,
    B_w2: jax.Array,
    B_w3: jax.Array,
    B_w4: jax.Array,
):
    del B_x
    x = A_x.reshape(S, D)
    any_spec = pl.BlockSpec(memory_space=pl.ANY)
    scratch = [
        pltpu.VMEM((S, D), BF16),
        pltpu.VMEM((G, D, 128), BF16),
        pltpu.VMEM((G, D, 128), BF16),
        pltpu.VMEM((G, D, 128), BF16),
        pltpu.VMEM((D, D), BF16),
        pltpu.VMEM((D, D), BF16),
        pltpu.VMEM((D, D), BF16),
        pltpu.VMEM((D, F), BF16),
        pltpu.VMEM((F, D), BF16),
        pltpu.VMEM((G, 128, D), BF16),
        pltpu.VMEM((G, 128, D), BF16),
        pltpu.VMEM((S, D), F32),
        pltpu.VMEM((S, D), F32),
        pltpu.VMEM((S, D), BF16),
        pltpu.VMEM((S, D), F32),
        pltpu.VMEM((D // 128, S + 2 * HPAD, 128), F32),
        pltpu.VMEM((NP, L, 128), BF16),
        pltpu.VMEM((NP, L, 128), BF16),
        pltpu.VMEM((NP, 128, L), BF16),
        pltpu.VMEM((NP, 128, L), BF16),
        pltpu.VMEM((NP, 128, L), BF16),
        pltpu.VMEM((2, G, L, 128), BF16),
        pltpu.VMEM((G, 128, 128), F32),
        pltpu.VMEM((G, 16, 128), F32),
        pltpu.VMEM((S, D), BF16),
        pltpu.VMEM((NP, NQT * HPG, QT), F32),
        pltpu.VMEM((NP * RC, D), BF16),
        pltpu.VMEM((TB, D), BF16),
        pltpu.VMEM((H,), BF16),
        pltpu.SMEM((H,), F32),
        pltpu.SMEM((2 * NP + 1,), F32),
        pltpu.SemaphoreType.DMA((len(X_PARTS),)),
        pltpu.SemaphoreType.DMA((G,)),
        pltpu.SemaphoreType.DMA((6,)),
        pltpu.SemaphoreType.DMA((NTB - 1 + NOUT,)),
    ]
    out = pl.pallas_call(
        _kernel,
        out_shape=jax.ShapeDtypeStruct((S, D), BF16),
        in_specs=[any_spec] * 10,
        out_specs=any_spec,
        scratch_shapes=scratch,
        compiler_params=pltpu.CompilerParams(vmem_limit_bytes=120 * 1024 * 1024),
    )(A_beta, x, A_wq, A_wk, A_wv, A_wo, B_w1, B_w2, B_w3, B_w4)
    return out.reshape(1, S, D)
```

```python
import functools

import jax
import jax.numpy as jnp
from jax import lax
import jax.experimental.pallas as pl
import jax.experimental.pallas.tpu as pltpu

S = 2048
D = 1024
H = 32
DH = 32
NSEG = 4
L = 512
F = 3584
G = 8
HPG = 4
QT = 128
NQT = L // QT
HQ = QT // 2
HPAD = 8
FC = 512
RC = L // G
NP = 4
LN_AT = (1, 2, 3, 4)
STAGES = "x0 g0 x1 x6|g1 g2|g3 g4|g5 x2|g6 g7 x3|"
TB = 256
NTB = S // TB
HEAD_T = "123"
FIRST_LN = [RC * int(c) for c in "00212111"]
LOOP_LN = [RC * int(c) for c in "01010101"]
OUT_R = 128
OUT_C = 512
OUT_PIECES = [(r, c) for r in range(0, TB, OUT_R) for c in range(0, D, OUT_C)]
NOUT = len(OUT_PIECES)
NHALF = 2
X_PARTS = ((0, QT), (QT, QT), (L, L // 2), (3 * L // 2, L // 2), (2 * L, L // 2), (5 * L // 2, 3 * L // 2), (L // 2, L // 2))
LOG2E = 1.4426950408889634
QSCALE = (DH ** -0.5) * LOG2E
MASK_BIAS = -1000000000.0 * LOG2E
GELU_C = 0.7978845608028654
SAFE_LOGIT = 40.0

F32 = jnp.float32
BF16 = jnp.bfloat16

NT = (((1,), (1,)), ((), ()))
SHIFTS = (-1, 1, -2, 2)
ORDER_FIRST = "S0 S1 P0 S2 P1 S3 P2 mr mu q L P3 c k L v W +S0 +S1 +P0 +S2 +P1 +S3 +P2 +mr +mu +q L +P3 +c +k L +v"
ORDER_LAST = "S0 S1 P0 S2 P1 S3 P2 mr wo P3 c +S3 +S2 +P3 +S1 +P2 +S0 +mr +P1 +P0 +c w1"
ORDER_TAIL = "o01 o23 m0 w01 w23"
ORDER_MID = "cp S0 S1 P0 S2 P1 S3 P2 mr mu q L P3 c k L wo v +S0 +S1 +P0 +S2 +P1 +S3 +P2 +mr +mu +q L +P3 +c +k L w1 +v"


def _ln(x):
    m = jnp.mean(x, axis=-1, keepdims=True)
    d = x - m
    v = jnp.mean(d * d, axis=-1, keepdims=True)
    return d * lax.rsqrt(v + 1e-05)


def _gelu(x):
    return 0.5 * x * (1.0 + jnp.tanh(GELU_C * (x + 0.044715 * (x * x * x))))


def _phi(t):
    return jnp.where(t > 0, t + 1.0, jnp.exp(t))


def _dot(a, b):
    return jnp.dot(a, b, preferred_element_type=F32)


def _kernel(beta_hbm, x_hbm, wq_hbm, wk_hbm, wv_hbm, wo_hbm, w1_hbm, w2_hbm, w3_hbm, w4_hbm,
            out_hbm,
            xin, wq, wk, wv, wo, w1, w2, w3, w4, wqt, wvt,
            xres, xmid, xn, ybuf, hbuf, kb, pkb, qt, pqt, vt, ob, mt, zr, obuf, shift, lnb, x1b, beta_in, beta, amax,
            sem_x, sem_g, sem_w, sem_out):

    def x_copy(s):
        rows = pl.ds(*X_PARTS[s])
        return pltpu.make_async_copy(x_hbm.at[rows], xin.at[rows], sem_x.at[s])

    def group_copies(g):
        return [pltpu.make_async_copy(src.at[:, pl.ds(g * 128, 128)], dst.at[g], sem_g.at[g])
                for src, dst in ((wk_hbm, wk), (wq_hbm, wq), (wv_hbm, wv))]

    def group_wait(g):
        for cp in group_copies(g):
            cp.wait()

    w_pairs = [(wo_hbm, wo), (w1_hbm, w1), (w2_hbm, w2), (w3_hbm, w3), (w4_hbm, w4), (beta_hbm, beta_in)]
    w_copies = [pltpu.make_async_copy(src, dst, sem_w.at[i]) for i, (src, dst) in enumerate(w_pairs)]
    cp_wo, cp_w1, cp_w2, cp_w3, cp_w4, cp_beta = w_copies

    def stage(i):
        for item in STAGES.split("|")[i].split():
            for cp in [x_copy(int(item[1]))] if item[0] == "x" else group_copies(int(item[1])):
                cp.start()

    cp_beta.start()
    stage(0)

    hbuf[:, 0:HPAD, :] = jnp.zeros((D // 128, HPAD, 128), F32)
    hbuf[:, HPAD + S:HPAD + S + HPAD, :] = jnp.zeros((D // 128, HPAD, 128), F32)
    xres[0:TB, :] = jnp.zeros((TB, D), F32)
    shift[...] = jnp.zeros(shift.shape, F32)
    amax[2 * NP] = 0.0

    def loop(lo, hi, fn):
        def body(i, c):
            fn(i)
            return c
        lax.fori_loop(lo, hi, body, 0)

    def aligned(i, n):
        return i if isinstance(i, int) else pl.multiple_of(i, n)

    def residual(layer, rows):
        return xin[rows, :].astype(F32) if layer == 0 else xres[rows, :]

    def seg_rows(s):
        return pl.ds(s * L if isinstance(s, int) else pl.multiple_of(s * L, L), L)

    def proj_k(b, s, g):
        k = _dot(xn[seg_rows(s), :], wk[g])
        kb[b] = k.astype(BF16)
        pkb[b] = _phi(k).astype(BF16)
        amax[2 * b] = mag = jnp.max(jnp.abs(k))
        return mag

    def swap_halves(x):
        return jnp.concatenate([pltpu.roll(x[:, c:c + QT], HQ, 1) for c in range(0, x.shape[1], QT)], axis=1)

    def scaled_q(q):
        qs = q * QSCALE
        heads = [qs[h * DH:(h + 1) * DH, :] for h in range(HPG)]
        return jnp.concatenate([x if h % 2 else swap_halves(x) for h, x in enumerate(heads)], axis=0).astype(BF16)

    def proj_q(b, s, w):
        q = lax.dot_general(w, xn[seg_rows(s), :], NT, preferred_element_type=F32)
        qt[b] = scaled_q(q)
        pqt[b] = _phi(q).astype(BF16)
        amax[2 * b + 1] = mag = jnp.max(jnp.abs(q))
        return mag

    def proj_v(b, s, w):
        v = lax.dot_general(w, xn[seg_rows(s), :], NT, preferred_element_type=F32)
        vt[b] = v.astype(BF16)

    def zero_after(mag):
        return 0 if mag is None else (mag < 0.0).astype(jnp.int32)

    def transposed(src, dst, g, mag=None):
        w = src[g ^ zero_after(mag)].T
        dst[g] = w
        return w

    def store_proj(op, b, rows, y, mags):
        if op == "k":
            kb[b, rows, :] = y.astype(BF16)
            pkb[b, rows, :] = _phi(y).astype(BF16)
            mags[2 * b].append(jnp.max(jnp.abs(y), axis=0, keepdims=True))
        elif op == "q":
            mags[2 * b + 1].append(jnp.max(jnp.abs(y), axis=0, keepdims=True))
            q = y.T
            qt[b, :, rows] = scaled_q(q)
            pqt[b, :, rows] = _phi(q).astype(BF16)
        else:
            vt[b, :, rows] = y.T.astype(BF16)

    def first_head():
        weights = {"k": wk, "q": wq, "v": wv}
        mags = [[] for _ in range(2 * NP)]

        def fresh_rows(c, groups):
            rows = pl.ds(c * QT, QT)
            xc = _ln(residual(0, rows)).astype(BF16)
            xn[rows, :] = xc
            for b in groups:
                for op in "kqv":
                    store_proj(op, b, rows, _dot(xc, weights[op][b]), mags)

        def known_rows(n, b):
            if str(b) in HEAD_T:
                proj_k(b, 0, b)
                proj_q(b, 0, transposed(wq, wqt, b))
                proj_v(b, 0, transposed(wv, wvt, b))
                return
            for op in "qvk":
                store_proj(op, b, pl.ds(0, n), _dot(xn[0:n, :], weights[op][b]), mags)

        cp_beta.wait()
        head_of = lax.broadcasted_iota(jnp.int32, (1, H), 1)
        betas = beta_in[...].astype(F32).reshape(1, H)
        for h in range(H):
            beta[h] = jnp.sum(jnp.where(head_of == h, betas, 0.0))
        x_copy(0).wait()
        stage(1)
        xn[0:QT, :] = _ln(residual(0, pl.ds(0, QT))).astype(BF16)
        x_copy(1).wait()
        group_wait(0)
        stage(2)
        known_rows(QT, 0)
        fresh_rows(1, [0])
        x_copy(6).wait()
        stage(3)
        fresh_rows(2, [0])
        fresh_rows(3, [0])
        group_wait(1)
        stage(4)
        known_rows(L, 1)
        group_wait(2)
        group_wait(3)
        stage(5)
        known_rows(L, 2)
        known_rows(L, 3)
        for i, m in enumerate(mags):
            if m:
                amax[i] = jnp.max(functools.reduce(jnp.maximum, m))

    def second_head():
        rows = pl.ds(S - TB, TB)
        xn[rows, :] = _ln(residual(1, rows)).astype(BF16)
        for b in range(NP):
            proj_q(b, 0, wqt[b])
            proj_k(b, 0, b)
            proj_v(b, 0, wvt[b])

    def out_wo(layer, s, r, n):
        rows = pl.ds(aligned(s * L + r, QT), n)
        rin = pl.ds(aligned(r, QT), n)
        o = jnp.concatenate([ob[s & 1, g, rin, :] for g in range(G)], axis=1)
        xm = residual(layer, rows) + _dot(o, wo[...])
        xmid[rows, :] = xm
        y = _ln(xm)
        ybuf[rows, :] = y
        return _ln(y).astype(BF16)

    def out_w1(s, r, n, yn):
        h = _gelu(_dot(yn, w1[...]))
        rows = pl.ds(aligned(HPAD + s * L + r, HPAD), n)
        for cb in range(D // 128):
            hbuf[cb, rows, :] = h[:, cb * 128:(cb + 1) * 128]

    def q_cols(b, queries):
        zero_blk = jnp.zeros((DH, QT), BF16)
        cols = []
        for h in range(HPG):
            blocks = [zero_blk] * HPG
            blocks[h] = qt[b, h * DH:(h + 1) * DH, queries]
            cols.append(jnp.concatenate(blocks, axis=0))
        return jnp.concatenate(cols, axis=1)

    def qk(b, i):
        return _dot(kb[b, 0:QT * i + HQ, :], q_cols(b, pl.ds(i * QT, QT)))

    def own_half(h, x, fill):
        lane = lax.broadcasted_iota(jnp.int32, x.shape, 1)
        return jnp.where(lane >= HQ if h % 2 else lane < HQ, x, fill)

    def qk_top(b, i):
        zero_half = jnp.zeros((DH, QT), jnp.uint32)
        blocks = [own_half(h, pltpu.bitcast(qt[b, h * DH:(h + 1) * DH, i * QT:(i + 1) * QT], jnp.uint32), 0)
                  for h in range(HPG)]
        pair = jnp.concatenate([jnp.concatenate(blocks[:2] + [zero_half], axis=0),
                                jnp.concatenate([zero_half] + blocks[2:], axis=0)], axis=1)
        return _dot(kb[b, QT * i + HQ:QT * (i + 1), :], pltpu.bitcast(pair, BF16))

    def causal_bias(nkeys, query):
        krow = lax.broadcasted_iota(jnp.int32, (nkeys, QT), 0)
        lane = lax.broadcasted_iota(jnp.int32, (nkeys, QT), 1)
        return jnp.where(krow > query(lane), MASK_BIAS, 0.0).astype(F32)

    def query_of(h):
        return (lambda lane: lane) if h % 2 else (lambda lane: (lane + HQ) & (QT - 1))

    def softmax_shift():
        scale = DH * QSCALE * 1.02
        safe = functools.reduce(jnp.logical_and,
                                [amax[2 * b] * amax[2 * b + 1] * scale <= SAFE_LOGIT for b in range(NP)],
                                amax[2 * NP] == 0.0)

        @pl.when(jnp.logical_not(safe))
        def _():
            amax[2 * NP] = 1.0

            def row_max(t):
                b = lax.shift_right_logical(t, 2)
                i = t & (NQT - 1)
                q0 = pl.multiple_of(i * QT, QT)
                st = _dot(kb[b], q_cols(b, pl.ds(q0, QT)))
                for h in range(HPG):
                    sc = st[:, h * QT:(h + 1) * QT] + causal_bias(L, lambda lane: q0 + query_of(h)(lane))
                    shift[b, pl.ds(i * HPG + h, 1), :] = jnp.max(sc, axis=0, keepdims=True)
            loop(0, NP * NQT, row_max)

    def probs(b, i):
        lo = qk(b, i)
        hi = qk_top(b, i)
        nd = QT * i
        shifts = [shift[b, i * HPG + h:i * HPG + h + 1, :] for h in range(HPG)]
        res = []
        for h in range(HPG):
            if h % 2 == 0:
                top = hi[:, (h // 2) * QT:(h // 2 + 1) * QT] + causal_bias(HQ, lambda lane: lane & (HQ - 1))
                top = jnp.exp2(top - own_half(h, shifts[h], shifts[h + 1]))
                top_sum = jnp.sum(top, axis=0, keepdims=True)
            sc = lo[:, h * QT:(h + 1) * QT]
            diag = sc[nd:, :] + causal_bias(HQ, query_of(h))
            p = jnp.exp2((diag if i == 0 else jnp.concatenate([sc[:nd, :], diag], axis=0)) - shifts[h])
            total = jnp.sum(p, axis=0, keepdims=True) + own_half(h, top_sum, 0.0)
            res.append((jnp.concatenate([p, own_half(h, top, 0.0)], axis=0).astype(BF16), total))
        return res

    def pv(b, i, ps):
        nk = QT * (i + 1)
        return [(_dot(vt[b, h * DH:(h + 1) * DH, 0:nk], ps[h][0]), ps[h][1]) for h in range(HPG)]

    def mem_read(b, g):
        mem = jnp.concatenate([mt[g], zr[g]], axis=0).astype(BF16)
        return _dot(mem, pqt[b])

    def mem_update(b, g):
        vaug = jnp.concatenate([vt[b], jnp.ones((16, L), BF16)], axis=0)
        upd = _dot(vaug, pkb[b])
        rh = lax.broadcasted_iota(jnp.int32, (144, 128), 0)
        ch = lax.broadcasted_iota(jnp.int32, (144, 128), 1) // DH
        upd = jnp.where(jnp.where(rh < 128, rh // DH, rh - 128) == ch, upd, 0.0)
        mt[g] = mt[g] + upd[:128]
        zr[g] = zr[g] + upd[128:]

    def combine(s, g, nd, res):
        rows = []
        for h in range(HPG):
            gate = jax.nn.sigmoid(jnp.full((1, L), beta[g * HPG + h], F32))
            l_h = jnp.concatenate([res[i][h][1] for i in range(NQT)], axis=1)
            o_h = jnp.concatenate([res[i][h][0] for i in range(NQT)], axis=1)
            c_dot = (1.0 - gate) / l_h
            c_mem = gate / (nd[128 + h:129 + h, :] + 1e-06)
            o_h = c_dot * o_h
            rows.append(c_mem * nd[h * DH:(h + 1) * DH, :] + (o_h if h % 2 else swap_halves(o_h)))
        ob[s & 1, g] = jnp.concatenate(rows, axis=0).T.astype(BF16)

    def run(layer, order, j, fresh):
        n = 2 * RC
        s = j >> 3
        last_rows = S - NP * RC
        state = [({}, {}, {}) for _ in range(NP)]
        shared = {}
        ops = [(op.lstrip("+"), base + op.count("+")) for base in range(0, NP, 2) for op in order.split()]
        for op, b in ops:
            ps, res, tmp = state[b]
            g = (j + b) & (G - 1)
            sn = (j + b + NP) >> 3
            gn = (j + b + NP) & (G - 1)
            if op[0] == "S":
                ps[int(op[1])] = probs(b, int(op[1]))
            elif op[0] == "P":
                res[int(op[1])] = pv(b, int(op[1]), ps[int(op[1])])
            elif op == "mr":
                tmp["nd"] = mem_read(b, g)
            elif op == "mu":
                mem_update(b, g)
            elif op == "wo":
                shared["yn"] = out_wo(layer, s - 1, g * RC, n)
            elif op == "w1":
                out_w1(s - 1, g * RC, n, shared["yn"])
            elif op == "q":
                shared["q"] = shared["mag"] = proj_q(b, sn, transposed(wq, wqt, gn, shared.get("q")) if fresh and str(gn) not in HEAD_T else wqt[gn])
            elif op == "k":
                shared["mag"] = proj_k(b, sn, gn)
            elif op == "v":
                proj_v(b, sn, transposed(wv, wvt, gn, shared["q"]) if fresh and str(gn) not in HEAD_T else wvt[gn])
            elif op == "L" and layer == 0:
                sizes = FIRST_LN if fresh and j == 0 else LOOP_LN
                idx = shared["ln"] = shared.get("ln", -1) + 1
                m, off = sizes[idx], sum(sizes[:idx])
                if m:
                    start = L if fresh and j == 0 else jnp.minimum((j + G + NP) * RC, last_rows)
                    after = zero_after(shared["mag"]) * RC if fresh else 0
                    y = _ln(residual(layer, pl.ds(pl.multiple_of(start + off - after, RC), m))).astype(BF16)
                    if fresh and j == 0:
                        xn[L + off:L + off + m, :] = y
                    else:
                        lnb[off:off + m, :] = y
            elif op == "cp" and layer == 0 and b == 0 and not fresh:
                rows = pl.ds(pl.multiple_of(jnp.minimum((j + G) * RC, last_rows), NP * RC), NP * RC)
                xn[rows, :] = lnb[...]
            elif op == "W" and layer == 0 and b == 0 and j == 0:
                for cp in [x_copy(2), x_copy(3)] + group_copies(6) + group_copies(7):
                    cp.wait()
            elif op == "c":
                combine(s, g, tmp["nd"], res)

    def attn_step(layer, order, it, fresh=False):
        softmax_shift()
        run(layer, order, it * NP if isinstance(it, int) else pl.multiple_of(it * NP, NP), fresh)

    def first_steps():
        group_wait(4)
        group_wait(5)
        x_copy(4).start()
        attn_step(0, ORDER_FIRST, 0, True)
        x_copy(4).wait()
        cp_wo.start()
        cp_w1.start()
        x_copy(5).start()
        attn_step(0, ORDER_FIRST, 1, True)

    def last_step(layer):
        attn_step(layer, ORDER_LAST, NSEG * G // NP - 1)
        yns = {}
        for op in ORDER_TAIL.split():
            r, n = int(op[1]) * QT, (int(op[-1]) - int(op[1]) + 1) * QT
            if op[0] == "m":
                if layer == 1:
                    mix(0)
            elif op[0] == "o":
                yns[op[1:]] = out_wo(layer, NSEG - 1, r, n)
            else:
                out_w1(NSEG - 1, r, n, yns[op[1:]])

    def out_copy(t):
        rows = pl.ds(aligned(t * TB, TB), TB)
        return pltpu.make_async_copy(obuf.at[rows], out_hbm.at[rows], sem_out.at[t])

    def out_piece(c):
        part = (pl.ds(S - TB + OUT_PIECES[c][0], OUT_R), pl.ds(OUT_PIECES[c][1], OUT_C))
        return pltpu.make_async_copy(obuf.at[part], out_hbm.at[part], sem_out.at[NTB - 1 + c])

    def mixed(t):
        hb = TB // NHALF
        for u in range(NHALF):
            ru = aligned(t * TB + u * hb, hb)
            parts = [hbuf[cb, pl.ds(ru + HPAD + SHIFTS[cb // 2], hb), :] for cb in range(D // 128)]
            x1 = ybuf[pl.ds(ru, hb), :] + _dot(jnp.concatenate(parts, axis=1).astype(BF16), w2[...])
            yield pl.ds(ru, hb), _ln(x1), xmid[pl.ds(ru, hb), :] + x1

    def mix(t):
        for u, (rows, xl, x) in enumerate(mixed(t)):
            x1b[u * xl.shape[0]:(u + 1) * xl.shape[0], :] = xl.astype(BF16)
            xmid[rows, :] = x

    def b_step(t, layer, ahead):
        r = aligned(t * TB, TB)
        if layer == 0:
            _, xls, xs = zip(*mixed(t))
            acc = jnp.concatenate(xs, axis=0)
            x1n = jnp.concatenate(xls, axis=0).astype(BF16)
        else:
            acc = xmid[pl.ds(r, TB), :]
        for ci in range(F // FC):
            if layer == 0 and ci in LN_AT:
                m = TB // len(LN_AT)
                off = LN_AT.index(ci) * m
                prev = pl.ds(pl.multiple_of(jnp.maximum(r - TB, 0) + off, m), m)
                normed = _ln(xres[prev, :])
                xn[prev, :] = normed.astype(BF16)
                pieces = [acc[:off], jnp.where(t < 0, normed, acc[off:off + m]), acc[off + m:]]
                acc = jnp.concatenate([p for p in pieces if p.shape[0]], axis=0)
            w3c = w3[:, ci * FC:(ci + 1) * FC]
            if layer == 0 and ci == 0:
                h = jnp.concatenate([_gelu(_dot(xl.astype(BF16), w3c)) for xl in xls], axis=0).astype(BF16)
            else:
                h = _gelu(_dot(x1n if layer == 0 else x1b[...], w3c)).astype(BF16)
            if ahead and ci == F // FC - 1:
                mix(t + 1)
            if layer == 1 and not ahead and ci == F // FC - 1:
                for c, (r0, c0) in enumerate(OUT_PIECES):
                    rows, cols = slice(r0, r0 + OUT_R), slice(c0, c0 + OUT_C)
                    piece = acc[rows, cols] + _dot(h[rows], w4[ci * FC:(ci + 1) * FC, cols])
                    obuf[pl.ds(r + r0, OUT_R), cols] = piece.astype(BF16)
                    out_piece(c).start()
                return
            acc = acc + _dot(h, w4[ci * FC:(ci + 1) * FC, :])
        if layer == 0:
            xres[pl.ds(r, TB), :] = acc
        else:
            obuf[pl.ds(r, TB), :] = acc.astype(BF16)
            out_copy(t).start()

    def layer_body(layer):
        mt[...] = jnp.zeros(mt.shape, F32)
        zr[...] = jnp.zeros(zr.shape, F32)

        (first_head if layer == 0 else second_head)()
        if layer == 1:
            loop(0, G // NP, lambda it: attn_step(layer, ORDER_FIRST, it))
        else:
            first_steps()
            cp_wo.wait()
            cp_w1.wait()
            x_copy(5).wait()
            for cp in (cp_w2, cp_w3, cp_w4):
                cp.start()
        loop(G // NP, NSEG * G // NP - 1, lambda it: attn_step(layer, ORDER_MID, it))
        if layer == 0:
            cp_w2.wait()
            cp_w3.wait()
            cp_w4.wait()
        last_step(layer)
        loop(0, NTB - layer, lambda t: b_step(t, layer, layer == 1))
        if layer == 1:
            b_step(NTB - 1, layer, False)

    for layer in range(2):
        layer_body(layer)

    for t in range(NTB - 1):
        out_copy(t).wait()
    for c in range(NOUT):
        out_piece(c).wait()


@jax.jit
def pallas_interleave_layers__memory_aug_infini_attn__mixer_s_mlp__prompt_kernel(
    A_x: jax.Array,
    A_wq: jax.Array,
    A_wk: jax.Array,
    A_wv: jax.Array,
    A_wo: jax.Array,
    A_beta: jax.Array,
    B_x: jax.Array,
    B_w1: jax.Array,
    B_w2: jax.Array,
    B_w3: jax.Array,
    B_w4: jax.Array,
):
    del B_x
    x = A_x.reshape(S, D)
    any_spec = pl.BlockSpec(memory_space=pl.ANY)
    scratch = [
        pltpu.VMEM((S, D), BF16),
        pltpu.VMEM((G, D, 128), BF16),
        pltpu.VMEM((G, D, 128), BF16),
        pltpu.VMEM((G, D, 128), BF16),
        pltpu.VMEM((D, D), BF16),
        pltpu.VMEM((D, D), BF16),
        pltpu.VMEM((D, D), BF16),
        pltpu.VMEM((D, F), BF16),
        pltpu.VMEM((F, D), BF16),
        pltpu.VMEM((G, 128, D), BF16),
        pltpu.VMEM((G, 128, D), BF16),
        pltpu.VMEM((S, D), F32),
        pltpu.VMEM((S, D), F32),
        pltpu.VMEM((S, D), BF16),
        pltpu.VMEM((S, D), F32),
        pltpu.VMEM((D // 128, S + 2 * HPAD, 128), F32),
        pltpu.VMEM((NP, L, 128), BF16),
        pltpu.VMEM((NP, L, 128), BF16),
        pltpu.VMEM((NP, 128, L), BF16),
        pltpu.VMEM((NP, 128, L), BF16),
        pltpu.VMEM((NP, 128, L), BF16),
        pltpu.VMEM((2, G, L, 128), BF16),
        pltpu.VMEM((G, 128, 128), F32),
        pltpu.VMEM((G, 16, 128), F32),
        pltpu.VMEM((S, D), BF16),
        pltpu.VMEM((NP, NQT * HPG, QT), F32),
        pltpu.VMEM((NP * RC, D), BF16),
        pltpu.VMEM((TB, D), BF16),
        pltpu.VMEM((H,), BF16),
        pltpu.SMEM((H,), F32),
        pltpu.SMEM((2 * NP + 1,), F32),
        pltpu.SemaphoreType.DMA((len(X_PARTS),)),
        pltpu.SemaphoreType.DMA((G,)),
        pltpu.SemaphoreType.DMA((6,)),
        pltpu.SemaphoreType.DMA((NTB - 1 + NOUT,)),
    ]
    out = pl.pallas_call(
        _kernel,
        out_shape=jax.ShapeDtypeStruct((S, D), BF16),
        in_specs=[any_spec] * 10,
        out_specs=any_spec,
        scratch_shapes=scratch,
        compiler_params=pltpu.CompilerParams(vmem_limit_bytes=120 * 1024 * 1024),
    )(A_beta, x, A_wq, A_wk, A_wv, A_wo, B_w1, B_w2, B_w3, B_w4)
    return out.reshape(1, S, D)
```
